```python
import jax
import jax.numpy as jnp

def _softmax(x, axis=-1):
    return jax.nn.softmax(x, axis=axis)

def _gelu(x):
    return jax.nn.gelu(x, approximate=True)

def _silu(x):
    return jax.nn.silu(x)

def _sigmoid(x):
    return jax.nn.sigmoid(x)

def _layernorm(x, axis=-1, eps=1e-05):
    m = jnp.mean(x, axis=axis, keepdims=True)
    v = jnp.var(x, axis=axis, keepdims=True)
    return (x - m) / jnp.sqrt(v + eps)

def _scatter_add(tgt, idx, src, axis=0):
    return tgt.at[idx].add(src)

def _segment_sum(src, seg, n):
    return jax.ops.segment_sum(src, seg, n)

class _Rng:

    def __init__(self, key):
        self._k = key

    def _next(self):
        self._k, sub = jax.random.split(self._k)
        return sub

    def normal(self, shape):
        return jax.random.normal(self._next(), shape, dtype=jnp.bfloat16)

    def randint(self, lo, hi, shape):
        return jax.random.randint(self._next(), shape, lo, hi, dtype=jnp.int32)

    def uniform(self, shape, lo=0.0, hi=1.0):
        return jax.random.uniform(self._next(), shape, jnp.bfloat16, lo, hi)

    def permutation(self, n):
        return jax.random.permutation(self._next(), n)
kernel_name = 'sequential_preLN__memory_aug_recurrent_mem_tr__moe_arch_mod__prompt'

def setup_inputs():
    _rng = _Rng(jax.random.key(int.from_bytes(__import__("os").urandom(4), "little")))
    _w = lambda a: (lambda t: t.astype(jnp.bfloat16) if jnp.issubdtype(t.dtype, jnp.floating) else t)(jnp.asarray(a))

    def _A_setup():
        B, S, Dm = (1, 2048, 512)
        H, Dh = (32, 128)
        M, seg = (8, 32)
        seg = min(seg, S)
        S = S // seg * seg
        return {'x': _w((lambda *s: _rng.normal(s) * 0.05)(B, S, Dm)), 'mem0': _w((lambda *s: _rng.normal(s) * 0.05)(B, M, Dm)), 'Wq': _w((lambda *s: _rng.normal(s) * 0.05)(Dm, H, Dh) * Dm ** (-0.5)), 'Wk': _w((lambda *s: _rng.normal(s) * 0.05)(Dm, H, Dh) * Dm ** (-0.5)), 'Wv': _w((lambda *s: _rng.normal(s) * 0.05)(Dm, H, Dh) * Dm ** (-0.5)), 'Wo': _w((lambda *s: _rng.normal(s) * 0.05)(H, Dh, Dm) * (H * Dh) ** (-0.5)), 'seg_len': seg}
    _A_in = _A_setup()

    def _B_setup():
        B, S, D, F, C = (1, 2048, 512, 1792, 2)
        return {'x': _w((lambda *s: _rng.normal(s) * 0.05)(B, S, D)), 'w_r': _w((lambda *s: _rng.normal(s) * 0.05)(D)), 'w_gate': _w((lambda *s: _rng.normal(s) * 0.05)(D, F)), 'w_up': _w((lambda *s: _rng.normal(s) * 0.05)(D, F)), 'w_down': _w((lambda *s: _rng.normal(s) * 0.05)(F, D))}
    _B_in = _B_setup()
    return {'A_x': _A_in['x'], 'A_mem0': _A_in['mem0'], 'A_Wq': _A_in['Wq'], 'A_Wk': _A_in['Wk'], 'A_Wv': _A_in['Wv'], 'A_Wo': _A_in['Wo'], 'A_seg_len': _A_in['seg_len'], 'B_x': _B_in['x'], 'B_w_r': _B_in['w_r'], 'B_w_gate': _B_in['w_gate'], 'B_w_up': _B_in['w_up'], 'B_w_down': _B_in['w_down']}

def reference(A_x, A_mem0, A_Wq, A_Wk, A_Wv, A_Wo, A_seg_len, B_x, B_w_r, B_w_gate, B_w_up, B_w_down):

    def _A_ref(x, mem0, Wq, Wk, Wv, Wo, seg_len):
        B, S, Dm = x.shape
        H, Dh = (Wq.shape[1], Wq.shape[2])
        M = mem0.shape[1]
        scale = Dh ** (-0.5)
        n_seg = S // seg_len
        L = M + seg_len
        idx = jnp.arange(L)
        mask = (idx[:, None] < M) | (idx[:, None] >= idx[None, :])
        mem = mem0
        outs = []
        for s in range(n_seg):
            xs = x[:, s * seg_len:(s + 1) * seg_len, :].copy()
            h = jnp.concatenate([mem, xs], axis=1)
            q = jnp.einsum('btd,dhe->bhte', h, Wq)
            k = jnp.einsum('btd,dhe->bhte', h, Wk)
            v = jnp.einsum('btd,dhe->bhte', h, Wv)
            scores = jnp.einsum('bhqe,bhke->bhqk', q, k) * scale
            scores = jnp.where(mask[None, None], scores, -1000000000.0)
            p = _softmax(scores, axis=-1)
            o = jnp.einsum('bhqk,bhke->bhqe', p, v)
            o = jnp.einsum('bhte,hed->btd', o, Wo)
            mem = o[:, :M, :].copy()
            outs.append(o[:, M:, :])
        return jnp.concatenate(outs, axis=1)

    def _B_ref(x, w_r, w_gate, w_up, w_down):
        B, S, D = x.shape
        C = 2
        r = x @ w_r
        idx = jnp.argsort(-r, axis=-1)[:, :C]
        idx_e = jnp.repeat(idx.reshape(B, C, 1), D, axis=2)
        x_sel = jnp.take_along_axis(x, idx_e, axis=1)
        g = _silu(x_sel @ w_gate)
        u = x_sel @ w_up
        y = g * u @ w_down
        r_sel = _sigmoid(jnp.take_along_axis(r, idx, axis=1))
        y = y * r_sel.reshape(B, C, 1)
        b_off = (jnp.arange(B) * S).reshape(B, 1)
        flat_idx = (idx + b_off).reshape(B * C)
        zero = (x * 0.0).reshape(B * S, D)
        upd = _scatter_add(zero, flat_idx, y.reshape(B * C, D), axis=0)
        return x + upd.reshape(B, S, D)
    x = A_x
    h = x + _A_ref(_layernorm(x, axis=-1), A_mem0, A_Wq, A_Wk, A_Wv, A_Wo, A_seg_len)
    h2 = h + _B_ref(_layernorm(h, axis=-1), B_w_r, B_w_gate, B_w_up, B_w_down)
    return h2
```

```python
import functools

import jax
import jax.numpy as jnp
import numpy as np
from jax import lax
from jax.experimental import pallas as pl
from jax.experimental.pallas import tpu as pltpu

F32 = jnp.float32
BF16 = jnp.bfloat16
U32 = jnp.uint32
EPS = 1e-05
MASKED = -1000000000.0
NN = (((1,), (0,)), ((), ()))
NT = (((1,), (1,)), ((), ()))
LANES = 128
HG = 16


def _rb(v):
    return v.astype(BF16).astype(F32)


def _layernorm(v):
    m = jnp.mean(v, axis=-1, keepdims=True)
    c = v - m
    var = jnp.mean(c * c, axis=-1, keepdims=True)
    sd = _rb(jnp.sqrt(_rb(_rb(var) + EPS)))
    return _rb(_rb(v - _rb(m)) / sd)


def _dot(a, b, dims=NN):
    return lax.dot_general(a, b, dims, preferred_element_type=F32)


def _kernel(x_hbm, mem0_ref, wq_hbm, wk_hbm, wv_hbm, wo_hbm, wr_ref, wg_hbm, wu_hbm, wd_hbm,
            out_hbm,
            x_v, xh_v, xt_v, stage, wqkv, wo_v, pre, wg_v, wu_v, wd_v,
            acc_v, h_v, r_v, out_v, sems, *, seg):
    S, D = x_v.shape
    M = mem0_ref.shape[0]
    H = wqkv.shape[1]
    Dh = wqkv.shape[3]
    n_seg = S // seg
    L = M + seg
    n_tail = M
    n_head = seg - n_tail
    scale = Dh ** (-0.5)
    n_grp = H // HG
    n_chunk = 3 * n_grp
    w_hbm = (wq_hbm, wk_hbm, wv_hbm)

    cp_x = pltpu.make_async_copy(x_hbm, x_v, sems.at[0])
    cp_w = [
        pltpu.make_async_copy(w_hbm[c // n_grp].at[:, pl.ds((c % n_grp) * HG, HG), :],
                              stage.at[c], sems.at[1 + c])
        for c in range(n_chunk)
    ]
    base = 1 + n_chunk
    n_col = D // LANES
    cp_wo = [
        pltpu.make_async_copy(wo_hbm.at[:, pl.ds(c * LANES, LANES)], wo_v.at[c], sems.at[base + c])
        for c in range(n_col)
    ]
    base += n_col
    cp_ffn = [
        pltpu.make_async_copy(src, dst, sems.at[base + i])
        for i, (src, dst) in enumerate(((wg_hbm, wg_v), (wu_hbm, wu_v), (wd_hbm, wd_v)))
    ]
    base += 3

    cp_x.start()
    cp_w[0].start()

    cp_x.wait()
    cp_w[1].start()

    def ln_body(i, carry):
        rows = pl.ds(pl.multiple_of(i * 2 * seg, 2 * seg), 2 * seg)
        xn = _layernorm(x_v[rows, :].astype(F32))
        xh_v[2 * i] = xn[:n_head]
        xh_v[2 * i + 1] = xn[seg:seg + n_head]
        tail = jnp.concatenate([xn[n_head:seg], xn[seg + n_head:]], axis=0)
        xt_v[pl.ds(pl.multiple_of(i * 2 * n_tail, 2 * n_tail), 2 * n_tail), :] = tail.astype(BF16)
        return carry

    lax.fori_loop(0, n_seg // 2, ln_body, 0)

    def repack(c, i):
        m, g = c // n_grp, c % n_grp
        v = stage[c, pl.ds(pl.multiple_of(i * 16, 16), 16)]
        v = pltpu.bitcast(v.reshape(16 * HG, Dh), U32)
        v = v.reshape(8, 2, HG // 2, Dh)
        a, b = v[:, 0], v[:, 1]
        even = jnp.swapaxes((a & 0xFFFF) | (b << 16), 0, 1)
        odd = jnp.swapaxes((a >> 16) | (b & np.uint32(0xFFFF0000)), 0, 1)
        rows = pl.ds(pl.multiple_of(i * 8, 8), 8)
        for j in range(HG // 2):
            wqkv[m, g * HG + 2 * j, rows, :] = even[j]
            wqkv[m, g * HG + 2 * j + 1, rows, :] = odd[j]

    def w_tile(m, h):
        return pltpu.bitcast(wqkv[m, h], BF16)

    def project_tail(c, i):
        m, h = c // n_grp, (c % n_grp) * HG + i
        pre[m, h] = _dot(xt_v[...], w_tile(m, h))

    n_rep = D // 16
    cp_w[0].wait()
    cp_w[2].start()
    lax.fori_loop(0, n_rep, lambda i, c: (repack(0, i), c)[1], 0)
    for c in range(n_chunk):
        if c + 1 < n_chunk:
            cp_w[c + 1].wait()
        if c + 3 < n_chunk:
            cp_w[c + 3].start()
        elif c + 3 == n_chunk:
            for cp in cp_wo:
                cp.start()

        def pre_body(i, carry, c=c):
            project_tail(c, i)
            if c + 1 < n_chunk:
                for t in range(n_rep // HG):
                    repack(c + 1, i * (n_rep // HG) + t)
            return carry

        lax.fori_loop(0, HG, pre_body, 0)

    for cp in cp_wo:
        cp.wait()
    for cp in cp_ffn:
        cp.start()

    acc_v[...] = jnp.zeros(acc_v.shape, F32)
    acc_v[0:M, :] = mem0_ref[...].astype(F32)
    r_v[...] = jnp.full(r_v.shape, -jnp.inf, F32)

    def finish_segment(sp, lane_id):
        rows = pl.ds(pl.multiple_of(sp * seg, seg), seg)
        h = _rb(x_v[rows, :].astype(F32) + _rb(acc_v[M:L, :]))
        hn = _layernorm(h)
        r = _rb(jnp.sum(hn * wr_ref[...].astype(F32), axis=-1, keepdims=True))
        h_v[rows, :] = h
        out_v[rows, :] = (h + hn).astype(BF16)
        lane = lax.broadcasted_iota(jnp.int32, r_v.shape, 1)
        r_v[...] = jnp.where(lane == lane_id, r, r_v[...])

    def step(s, carry):
        finish_segment(jnp.maximum(s - 1, 0), s - 1)
        lhs = jnp.concatenate([acc_v[0:M, :], xh_v[s]], axis=0).astype(BF16)
        tail = pl.ds(pl.multiple_of(s * n_tail, n_tail), n_tail)
        qi = lax.broadcasted_iota(jnp.int32, (L, L), 0)
        ki = lax.broadcasted_iota(jnp.int32, (L, L), 1)
        visible = (qi < M) | (qi >= ki)

        def proj(m, h):
            return jnp.concatenate([_dot(lhs, w_tile(m, h)), pre[m, h, tail, :]], axis=0)

        q, k, v, e, inv, o = {}, {}, {}, {}, {}, {}
        acc = None
        lag_s, lag_v, lag_pv, lag_o = 2, 6, 8, 12
        for i in range(H + lag_o):
            if i < H:
                q[i] = proj(0, i)
                k[i] = proj(1, i)
            j = i - lag_s
            if 0 <= j < H:
                sc = jnp.where(visible, _dot(q.pop(j), k.pop(j), NT) * scale, MASKED)
                ex = jnp.exp(sc - jnp.max(sc, axis=-1, keepdims=True))
                e[j] = ex
                inv[j] = 1.0 / jnp.sum(ex, axis=-1, keepdims=True)
            j = i - lag_v
            if 0 <= j < H:
                v[j] = proj(2, j)
            j = i - lag_pv
            if 0 <= j < H:
                o[j] = _dot(e.pop(j), v.pop(j)) * inv.pop(j)
            j = i - lag_o
            if 0 <= j < H:
                wo = jnp.concatenate(
                    [wo_v[c, j * Dh:(j + 1) * Dh, :] for c in range(n_col)], axis=1)
                y = _dot(o.pop(j), wo)
                acc = y if acc is None else acc + y
        acc_v[...] = acc
        return carry

    lax.fori_loop(0, n_seg, step, 0)
    finish_segment(n_seg - 1, n_seg - 1)
    cp_out = pltpu.make_async_copy(out_v, out_hbm, sems.at[base])
    cp_out.start()

    r = r_v[...]
    pos = (lax.broadcasted_iota(jnp.int32, r.shape, 1) * seg
           + lax.broadcasted_iota(jnp.int32, r.shape, 0))
    r = jnp.where(r != r, -jnp.inf, r)
    big = r.shape[0] * r.shape[1]
    r0 = jnp.max(r)
    i0 = jnp.min(jnp.where(r == r0, pos, big))
    rest = jnp.where(pos == i0, -jnp.inf, r)
    r1 = jnp.max(rest)
    i1 = jnp.min(jnp.where((rest == r1) & (pos != i0), pos, big))
    i0 = jnp.clip(i0, 0, S - 1)
    i1 = jnp.clip(i1, 0, S - 1)

    first = lax.broadcasted_iota(jnp.int32, (8, D), 0) == 0
    h_sel = jnp.where(first, h_v[pl.ds(i0, 1), :], h_v[pl.ds(i1, 1), :])
    hn_sel = _layernorm(h_sel)
    r_sel = _rb(jnp.sum(hn_sel * wr_ref[...].astype(F32), axis=-1, keepdims=True))
    for cp in cp_ffn:
        cp.wait()
    g = _rb(_dot(hn_sel, wg_v[...]))
    u = _rb(_dot(hn_sel, wu_v[...]))
    g = _rb(g * _rb(jax.nn.sigmoid(g)))
    y = _rb(_dot(_rb(g * u), wd_v[...]))
    y = _rb(y * _rb(jax.nn.sigmoid(r_sel)))
    new = h_sel + _rb(hn_sel + y)

    cp_out.wait()
    tile = 16
    for t, idx in enumerate((i0, i1)):
        start = pl.multiple_of((idx // tile) * tile, tile)
        rows = pl.ds(start, tile)
        hit = lax.broadcasted_iota(jnp.int32, (tile, D), 0) == idx - start
        out_v[rows, :] = jnp.where(hit, new[t:t + 1], out_v[rows, :].astype(F32)).astype(BF16)
        cp = pltpu.make_async_copy(out_v.at[rows], out_hbm.at[rows], sems.at[base])
        cp.start()
        cp.wait()


@functools.partial(jax.jit, static_argnames=("A_seg_len",))
def pallas_sequential_preLN__memory_aug_recurrent_mem_tr__moe_arch_mod__prompt_kernel(
    A_x: jax.Array,
    A_mem0: jax.Array,
    A_Wq: jax.Array,
    A_Wk: jax.Array,
    A_Wv: jax.Array,
    A_Wo: jax.Array,
    A_seg_len: int,
    B_x: jax.Array,
    B_w_r: jax.Array,
    B_w_gate: jax.Array,
    B_w_up: jax.Array,
    B_w_down: jax.Array,
):
    del B_x
    B, S, D = A_x.shape
    M = A_mem0.shape[1]
    _, H, Dh = A_Wq.shape
    F = B_w_gate.shape[1]
    seg = int(A_seg_len)
    n_seg = S // seg
    assert B == 1 and Dh == LANES and n_seg <= LANES and S % (2 * seg) == 0 and H % HG == 0

    hbm = pl.BlockSpec(memory_space=pl.ANY)
    vmem = pl.BlockSpec(memory_space=pltpu.VMEM)
    n_chunk = 3 * (H // HG)
    out = pl.pallas_call(
        functools.partial(_kernel, seg=seg),
        out_shape=jax.ShapeDtypeStruct((S, D), BF16),
        in_specs=[hbm, vmem, hbm, hbm, hbm, hbm, vmem, hbm, hbm, hbm],
        out_specs=hbm,
        scratch_shapes=[
            pltpu.VMEM((S, D), BF16),
            pltpu.VMEM((n_seg, seg - M, D), F32),
            pltpu.VMEM((n_seg * M, D), BF16),
            pltpu.VMEM((n_chunk, D, HG, Dh), BF16),
            pltpu.VMEM((3, H, D // 2, Dh), U32),
            pltpu.VMEM((D // LANES, H * Dh, LANES), BF16),
            pltpu.VMEM((3, H, n_seg * M, Dh), F32),
            pltpu.VMEM((D, F), BF16),
            pltpu.VMEM((D, F), BF16),
            pltpu.VMEM((F, D), BF16),
            pltpu.VMEM((M + seg, D), F32),
            pltpu.VMEM((S, D), F32),
            pltpu.VMEM((seg, LANES), F32),
            pltpu.VMEM((S, D), BF16),
            pltpu.SemaphoreType.DMA((n_chunk + D // LANES + 5,)),
        ],
        compiler_params=pltpu.CompilerParams(vmem_limit_bytes=110 * 1024 * 1024),
        name="rmt_mod_block",
    )(
        A_x.reshape(S, D), A_mem0.reshape(M, D), A_Wq, A_Wk, A_Wv, A_Wo.reshape(H * Dh, D),
        B_w_r.reshape(1, D), B_w_gate, B_w_up, B_w_down,
    )
    return out.reshape(B, S, D)
```

```python
import functools

import jax
import jax.numpy as jnp
import numpy as np
from jax import lax
from jax.experimental import pallas as pl
from jax.experimental.pallas import tpu as pltpu

F32 = jnp.float32
BF16 = jnp.bfloat16
U32 = jnp.uint32
EPS = 1e-05
MASKED = -1000000000.0
NN = (((1,), (0,)), ((), ()))
NT = (((1,), (1,)), ((), ()))
LANES = 128
HG = 8


def _rb(v):
    return v.astype(BF16).astype(F32)


def _layernorm(v):
    m = jnp.mean(v, axis=-1, keepdims=True)
    c = v - m
    var = jnp.mean(c * c, axis=-1, keepdims=True)
    sd = _rb(jnp.sqrt(_rb(_rb(var) + EPS)))
    return _rb(_rb(v - _rb(m)) / sd)


def _dot(a, b, dims=NN):
    return lax.dot_general(a, b, dims, preferred_element_type=F32)


def _kernel(x_hbm, mem0_ref, wq_hbm, wk_hbm, wv_hbm, wo_hbm, wr_ref, wg_hbm, wu_hbm, wd_hbm,
            out_hbm,
            x_v, xt_raw, xh_v, xt_v, stage, w_even, w_odd, wo_raw, wo_v, wg_v, wu_v, wd_v,
            acc_v, h_v, r_v, out_v, sem_w, sem_aux, sem):
    n_seg, seg, D = x_v.shape
    S = n_seg * seg
    M = mem0_ref.shape[0]
    H, Dh, _ = wo_raw.shape
    L = M + seg
    n_tail = xt_raw.shape[1]
    n_head = seg - n_tail
    scale = Dh ** (-0.5)
    n_grp = H // HG
    n_chunk = 3 * n_grp
    n_x = 2 * n_grp
    x_per = n_seg // n_x
    w_hbm = (wq_hbm, wk_hbm, wv_hbm)

    def w_copy(m, c):
        heads = pl.ds(pl.multiple_of((c - m * n_grp) * HG, HG), HG)
        return pltpu.make_async_copy(w_hbm[m].at[:, heads, :], stage.at[c], sem_w.at[c])

    def per_matrix(c, fn):
        for m in range(3):
            pl.when(c // n_grp == m)(functools.partial(lambda m: fn(w_copy(m, c)), m))

    def x_copy(c):
        segs = pl.ds(c * x_per, x_per)
        return pltpu.make_async_copy(x_hbm.at[segs], x_v.at[segs], sem_aux.at[c])

    def wo_copy(c):
        heads = pl.ds((c - n_x) * HG, HG)
        return pltpu.make_async_copy(wo_hbm.at[heads], wo_raw.at[heads], sem_aux.at[c])

    cp_tail = pltpu.make_async_copy(x_hbm.at[:, pl.ds(n_head, n_tail), :], xt_raw, sem.at[0])
    cp_ffn = [
        pltpu.make_async_copy(src, dst, sem.at[1 + i])
        for i, (src, dst) in enumerate(((wg_hbm, wg_v), (wu_hbm, wu_v), (wd_hbm, wd_v)))
    ]

    cp_tail.start()
    w_copy(0, 0).start()

    cp_tail.wait()
    w_copy(0, 1).start()
    x_copy(0).start()
    ln_per = 16

    def ln_body(i, carry):
        xn = _layernorm(xt_raw[pl.ds(i * ln_per, ln_per)].astype(F32).reshape(ln_per * n_tail, D))
        half = ln_per * n_tail // 2
        xt_v[pl.ds(pl.multiple_of(i * half, half), half), :] = pltpu.bitcast(xn.astype(BF16), U32)
        return carry

    lax.fori_loop(0, n_seg // ln_per, ln_body, 0)

    w_buf = (w_even, w_odd)

    def repack(src, dst, slot, i):
        v = stage[src, pl.ds(i * 16, 16)]
        v = pltpu.bitcast(v.reshape(16 * HG, Dh), U32)
        v = jnp.swapaxes(v.reshape(8, HG, Dh), 0, 1)
        rows = pl.ds(i * 8, 8) if isinstance(i, int) else pl.ds(pl.multiple_of(i * 8, 8), 8)
        for j in range(HG // 2):
            a, b = v[j], v[HG // 2 + j]
            dst[slot, 2 * j, rows, :] = (a & 0xFFFF) | (b << 16)
            dst[slot, 2 * j + 1, rows, :] = (a >> 16) | (b & np.uint32(0xFFFF0000))

    def w_tile(j):
        c = j // HG
        return pltpu.bitcast(w_buf[c % 2][c // 2, j % HG], BF16)

    n_rep = D // 16
    w_copy(0, 0).wait()
    w_copy(0, 2).start()
    x_copy(1).start()
    lax.fori_loop(0, n_rep, lambda i, c: (repack(0, w_even, 0, i), c)[1], 0, unroll=4)

    def pair_body(p, carry, *, with_x):
        for par in range(2):
            c = 2 * p + par
            per_matrix(c + 1, lambda cp: cp.wait())
            per_matrix(c + 3, lambda cp: cp.start())
            if with_x:
                x_copy(c).wait()
                pl.when(c + 2 < n_x)(lambda: x_copy(c + 2).start())
                pl.when(c + 2 >= n_x)(lambda: wo_copy(c + 2).start())
            else:
                wo_copy(c).wait()
                pl.when(c + 2 < n_chunk)(lambda: wo_copy(c + 2).start())

            if not with_x:
                for t in range(HG):
                    h = (c - n_x) * HG + t
                    wo_v[h] = pltpu.bitcast(wo_raw[h], U32)
            src = jnp.minimum(c + 1, n_chunk - 1)
            n_part = n_rep // HG
            part = n_seg // n_part
            for i in range(HG):
                y = _dot(pltpu.bitcast(xt_v[...], BF16), pltpu.bitcast(w_buf[par][p, i], BF16))
                y = y.reshape(n_seg, n_tail, Dh).astype(BF16)
                for t in range(n_part):
                    repack(src, w_buf[1 - par], p + par, i * n_part + t)
                    stage[c, pl.ds(i * n_seg + t * part, part)] = y[t * part:(t + 1) * part]
        return carry

    lax.fori_loop(0, n_x // 2, functools.partial(pair_body, with_x=True), 0)
    lax.fori_loop(n_x // 2, n_chunk // 2, functools.partial(pair_body, with_x=False), 0)
    for cp in cp_ffn:
        cp.start()

    acc_v[...] = jnp.zeros(acc_v.shape, F32)
    acc_v[0:M, :] = mem0_ref[...].astype(F32)
    r_v[...] = jnp.full(r_v.shape, -jnp.inf, F32)

    def norm_head(sg):
        xh_v[...] = _layernorm(x_v[sg].astype(F32)[:n_head])

    norm_head(0)

    def route(hn):
        w = wr_ref[...].astype(F32)
        w = jnp.concatenate([w[i:i + 1] for i in range(w.shape[0])], axis=1)
        return _rb(jnp.sum(hn * w, axis=-1, keepdims=True))

    early = (n_seg - 2) * seg
    cp_early = pltpu.make_async_copy(out_v.at[pl.ds(0, early)], out_hbm.at[pl.ds(0, early)], sem.at[4])
    cp_late = pltpu.make_async_copy(out_v.at[pl.ds(early, S - early)],
                                    out_hbm.at[pl.ds(early, S - early)], sem.at[5])

    def finish_segment(sp, lane_id):
        rows = pl.ds(pl.multiple_of(sp * seg, seg), seg)
        h = _rb(x_v[sp].astype(F32) + _rb(acc_v[M:L, :]))
        hn = _layernorm(h)
        r = route(hn)
        h_v[rows, :] = h
        out_v[rows, :] = (h + hn).astype(BF16)
        lane = lax.broadcasted_iota(jnp.int32, r_v.shape, 1)
        r_v[...] = jnp.where(lane == lane_id, r, r_v[...])

    def step(s, carry):
        pl.when(s == n_seg - 1)(cp_early.start)
        finish_segment(jnp.maximum(s - 1, 0), s - 1)
        lhs = jnp.concatenate([acc_v[0:M, :], xh_v[...]], axis=0).astype(BF16)
        norm_head(jnp.minimum(s + 1, n_seg - 1))
        qi = lax.broadcasted_iota(jnp.int32, (L, L), 0)
        ki = lax.broadcasted_iota(jnp.int32, (L, L), 1)
        visible = (qi < M) | (qi >= ki)

        def proj(m, h):
            j = m * H + h
            tail = stage[j // HG, (j % HG) * n_seg + s].astype(F32)
            return jnp.concatenate([_dot(lhs, w_tile(j)), tail], axis=0)

        q, k, v, e, inv, o = {}, {}, {}, {}, {}, {}
        acc = None
        lag_s, lag_v, lag_pv, lag_o = 2, 6, 8, 12
        for i in range(H + lag_o):
            if i < H:
                q[i] = proj(0, i)
                k[i] = proj(1, i)
            j = i - lag_s
            if 0 <= j < H:
                sc = jnp.where(visible, _dot(q.pop(j), k.pop(j), NT) * scale, MASKED)
                ex = jnp.exp(sc - jnp.max(sc, axis=-1, keepdims=True))
                e[j] = ex
                inv[j] = 1.0 / jnp.sum(ex, axis=-1, keepdims=True)
            j = i - lag_v
            if 0 <= j < H:
                v[j] = proj(2, j)
            j = i - lag_pv
            if 0 <= j < H:
                o[j] = _dot(e.pop(j), v.pop(j)) * inv.pop(j)
            j = i - lag_o
            if 0 <= j < H:
                y = _dot(o.pop(j), pltpu.bitcast(wo_v[j], BF16))
                acc = y if acc is None else acc + y
        acc_v[...] = acc
        return carry

    lax.fori_loop(0, n_seg, step, 0)
    finish_segment(n_seg - 1, n_seg - 1)
    cp_late.start()

    r = r_v[...]
    pos = (lax.broadcasted_iota(jnp.int32, r.shape, 1) * seg
           + lax.broadcasted_iota(jnp.int32, r.shape, 0))
    r = jnp.where(r != r, -jnp.inf, r)
    big = r.shape[0] * r.shape[1]
    r0 = jnp.max(r)
    i0 = jnp.min(jnp.where(r == r0, pos, big))
    rest = jnp.where(pos == i0, -jnp.inf, r)
    r1 = jnp.max(rest)
    i1 = jnp.min(jnp.where((rest == r1) & (pos != i0), pos, big))
    i0 = jnp.clip(i0, 0, S - 1)
    i1 = jnp.clip(i1, 0, S - 1)

    first = lax.broadcasted_iota(jnp.int32, (8, D), 0) == 0
    h_sel = jnp.where(first, h_v[pl.ds(i0, 1), :], h_v[pl.ds(i1, 1), :])
    hn_sel = _layernorm(h_sel)
    r_sel = route(hn_sel)
    for cp in cp_ffn:
        cp.wait()
    g = _rb(_dot(hn_sel, wg_v[...]))
    u = _rb(_dot(hn_sel, wu_v[...]))
    g = _rb(g * _rb(jax.nn.sigmoid(g)))
    y = _rb(_dot(_rb(g * u), wd_v[...]))
    y = _rb(y * _rb(jax.nn.sigmoid(r_sel)))
    new = h_sel + _rb(hn_sel + y)

    cp_early.wait()
    cp_late.wait()
    tile = 16
    fix = []
    for t, idx in enumerate((i0, i1)):
        start = pl.multiple_of((idx // tile) * tile, tile)
        rows = pl.ds(start, tile)
        hit = lax.broadcasted_iota(jnp.int32, (tile, D), 0) == idx - start
        out_v[rows, :] = jnp.where(hit, new[t:t + 1], out_v[rows, :].astype(F32)).astype(BF16)
        fix.append(pltpu.make_async_copy(out_v.at[rows], out_hbm.at[rows], sem.at[4 + t]))
    two_tiles = i0 // tile != i1 // tile
    fix[0].start()
    pl.when(two_tiles)(fix[1].start)
    fix[0].wait()
    pl.when(two_tiles)(fix[1].wait)


@functools.partial(jax.jit, static_argnames=("A_seg_len",))
def pallas_sequential_preLN__memory_aug_recurrent_mem_tr__moe_arch_mod__prompt_kernel(
    A_x: jax.Array,
    A_mem0: jax.Array,
    A_Wq: jax.Array,
    A_Wk: jax.Array,
    A_Wv: jax.Array,
    A_Wo: jax.Array,
    A_seg_len: int,
    B_x: jax.Array,
    B_w_r: jax.Array,
    B_w_gate: jax.Array,
    B_w_up: jax.Array,
    B_w_down: jax.Array,
):
    del B_x
    B, S, D = A_x.shape
    M = A_mem0.shape[1]
    _, H, Dh = A_Wq.shape
    F = B_w_gate.shape[1]
    seg = int(A_seg_len)
    n_seg = S // seg
    assert B == 1 and Dh == LANES and n_seg <= LANES and S % (2 * seg) == 0 and H % HG == 0

    hbm = pl.BlockSpec(memory_space=pl.ANY)
    vmem = pl.BlockSpec(memory_space=pltpu.VMEM)
    n_chunk = 3 * (H // HG)
    out = pl.pallas_call(
        _kernel,
        out_shape=jax.ShapeDtypeStruct((S, D), BF16),
        in_specs=[hbm, vmem, hbm, hbm, hbm, hbm, vmem, hbm, hbm, hbm],
        out_specs=hbm,
        scratch_shapes=[
            pltpu.VMEM((n_seg, seg, D), BF16),
            pltpu.VMEM((n_seg, M, D), BF16),
            pltpu.VMEM((seg - M, D), F32),
            pltpu.VMEM((n_seg * M // 2, D), U32),
            pltpu.VMEM((n_chunk, D, HG, Dh), BF16),
            pltpu.VMEM((n_chunk // 2 + 1, HG, D // 2, Dh), U32),
            pltpu.VMEM((n_chunk // 2, HG, D // 2, Dh), U32),
            pltpu.VMEM((H, Dh, D), BF16),
            pltpu.VMEM((H, Dh // 2, D), U32),
            pltpu.VMEM((D, F), BF16),
            pltpu.VMEM((D, F), BF16),
            pltpu.VMEM((F, D), BF16),
            pltpu.VMEM((M + seg, D), F32),
            pltpu.VMEM((S, D), F32),
            pltpu.VMEM((seg, LANES), F32),
            pltpu.VMEM((S, D), BF16),
            pltpu.SemaphoreType.DMA((n_chunk,)),
            pltpu.SemaphoreType.DMA((n_chunk,)),
            pltpu.SemaphoreType.DMA((6,)),
        ],
        compiler_params=pltpu.CompilerParams(vmem_limit_bytes=110 * 1024 * 1024),
        name="rmt_mod_block",
    )(
        A_x.reshape(n_seg, seg, D), A_mem0.reshape(M, D), A_Wq, A_Wk, A_Wv, A_Wo,
        B_w_r.reshape(D // LANES, LANES), B_w_gate, B_w_up, B_w_down,
    )
    return out.reshape(B, S, D)
```

```python
import functools

import jax
import jax.numpy as jnp
import numpy as np
from jax import lax
from jax.experimental import pallas as pl
from jax.experimental.pallas import tpu as pltpu

F32 = jnp.float32
BF16 = jnp.bfloat16
U32 = jnp.uint32
EPS = 1e-05
MASKED = -1000000000.0
LOG2E = 1.4426950408889634
NN = (((1,), (0,)), ((), ()))
NT = (((1,), (1,)), ((), ()))
LANES = 128
HG = 8
LATE = 2
UNROLL = 4


def _rb(v):
    return v.astype(BF16).astype(F32)


def _layernorm(v):
    m = jnp.mean(v, axis=-1, keepdims=True)
    c = v - m
    var = jnp.mean(c * c, axis=-1, keepdims=True)
    sd = _rb(jnp.sqrt(_rb(_rb(var) + EPS)))
    return _rb(_rb(v - _rb(m)) / sd)


def _recip(v):
    r = pl.reciprocal(v, approx=True)
    return r + r * (1.0 - v * r)


def _dot(a, b, dims=NN):
    return lax.dot_general(a, b, dims, preferred_element_type=F32)


def _issue_order(n_heads):
    lag_v, lag_o = 6, 10
    cost = {"q": 32, "k": 32, "v": 32, "s": 10, "p": 10, "o": 40}
    lat_mxu, lat_softmax = 240, 500
    needs = {"s": (("k", lat_mxu),), "p": (("v", lat_mxu), ("s", lat_softmax)), "o": (("p", lat_mxu),)}
    proj = []
    for i in range(n_heads + lag_v):
        proj += [("q", i), ("k", i)] if i < n_heads else []
        proj += [("v", i - lag_v)] if i >= lag_v else []
    nxt = {"s": 0, "p": 0, "o": 0}
    done, order, now = {}, [], 0

    def ready_at(kind):
        h = nxt[kind]
        if h == n_heads or any((d, h) not in done for d, _ in needs[kind]):
            return None
        return max(done[d, h] + lat for d, lat in needs[kind])

    while len(order) < 6 * n_heads:
        at = {kind: ready_at(kind) for kind in nxt}
        if proj and ("v", min(nxt["o"] + lag_o, n_heads - 1)) not in done:
            at["o"] = None
        kinds = [kind for kind in nxt if at[kind] is not None]
        if not proj:
            now = max(now, min(at[kind] for kind in kinds))
        kinds = [kind for kind in kinds if at[kind] <= now]
        if kinds:
            op = (kinds[0], nxt[kinds[0]])
            nxt[kinds[0]] += 1
        else:
            op = proj.pop(0)
        now += cost[op[0]]
        done[op] = now
        order.append(op)
    return order


def _kernel(x_hbm, mem0_ref, wq_hbm, wk_hbm, wv_hbm, wo_hbm, wr_ref, wg_hbm, wu_hbm, wd_hbm,
            out_hbm,
            x_v, xt_raw, xh_v, xt_v, stage, w_even, w_odd, wo_raw, wg_v, wu_v, wd_v,
            acc_v, h_v, out_v, sem_w, sem_wo, sem):
    n_seg, seg, D = x_v.shape
    S = n_seg * seg
    M = mem0_ref.shape[0]
    H, Dh, _ = wo_raw.shape
    L = M + seg
    n_tail = xt_raw.shape[1]
    n_head = seg - n_tail
    scale = Dh ** (-0.5)
    n_grp = H // HG
    n_chunk = 3 * n_grp
    n_ahead = n_chunk - LATE
    c_wo = n_ahead - n_grp
    n_col = D // LANES
    w_hbm = (wq_hbm, wk_hbm, wv_hbm)

    def w_copy(m, c):
        heads = pl.ds(pl.multiple_of((c - m * n_grp) * HG, HG), HG)
        return pltpu.make_async_copy(w_hbm[m].at[:, heads, :], stage.at[c], sem_w.at[c])

    def per_matrix(c, fn):
        for m in range(3):
            pl.when(c // n_grp == m)(functools.partial(lambda m: fn(w_copy(m, c)), m))

    def wo_copy(g):
        heads = pl.ds(g * HG, HG)
        return pltpu.make_async_copy(wo_hbm.at[heads], wo_raw.at[heads], sem_wo.at[g])

    cp_x = pltpu.make_async_copy(x_hbm, x_v, sem.at[6])
    cp_tail = pltpu.make_async_copy(x_hbm.at[:, pl.ds(n_head, n_tail), :], xt_raw, sem.at[0])
    cp_ffn = [
        pltpu.make_async_copy(src, dst, sem.at[1 + i])
        for i, (src, dst) in enumerate(((wg_hbm, wg_v), (wu_hbm, wu_v), (wd_hbm, wd_v)))
    ]

    cp_tail.start()
    w_copy(0, 0).start()

    cp_tail.wait()
    w_copy(0, 1).start()
    ln_per = 16

    def ln_body(i, carry):
        xn = _layernorm(xt_raw[pl.ds(i * ln_per, ln_per)].astype(F32).reshape(ln_per * n_tail, D))
        half = ln_per * n_tail // 2
        xt_v[pl.ds(pl.multiple_of(i * half, half), half), :] = pltpu.bitcast(xn.astype(BF16), U32)
        return carry

    lax.fori_loop(0, n_seg // ln_per, ln_body, 0)

    w_buf = (w_even, w_odd)

    def repack(src, dst, slot, i):
        v = stage[src, pl.ds(i * 16, 16)]
        v = pltpu.bitcast(v.reshape(16 * HG, Dh), U32)
        v = jnp.swapaxes(v.reshape(8, HG, Dh), 0, 1)
        rows = pl.ds(i * 8, 8) if isinstance(i, int) else pl.ds(pl.multiple_of(i * 8, 8), 8)
        for j in range(HG // 2):
            a, b = v[j], v[HG // 2 + j]
            dst[slot, 2 * j, rows, :] = (a & 0xFFFF) | (b << 16)
            dst[slot, 2 * j + 1, rows, :] = (a >> 16) | (b & np.uint32(0xFFFF0000))

    def w_tile(j):
        c = j // HG
        return pltpu.bitcast(w_buf[c % 2][c // 2, j % HG], BF16)

    n_rep = D // 16
    w_copy(0, 0).wait()
    w_copy(0, 2).start()
    lax.fori_loop(0, n_rep, lambda i, c: (repack(0, w_even, 0, i), c)[1], 0, unroll=4)

    def pair_body(p, carry, *, with_wo):
        for par in range(2):
            c = 2 * p + par
            per_matrix(c + 1, lambda cp: cp.wait())
            per_matrix(c + 3, lambda cp: cp.start())
            if with_wo:
                wo_copy(c - c_wo).wait()
                pl.when(c == c_wo)(cp_x.start)
            else:
                g = c - (c_wo - n_grp)
                pl.when(g >= 0)(lambda: wo_copy(g).start())
            src = jnp.minimum(c + 1, n_ahead)
            n_part = n_rep // HG
            part = n_seg // n_part
            for i in range(HG):
                if with_wo:
                    w = pltpu.bitcast(wo_raw[(c - c_wo) * HG + i], U32)
                    w_buf[par][jnp.minimum((n_chunk - c_wo) // 2 + p, 2 * n_grp - 1), i] = jnp.concatenate(
                        [w[:, t * LANES:(t + 1) * LANES] for t in range(n_col)], axis=0)
                y = _dot(pltpu.bitcast(xt_v[...], BF16), pltpu.bitcast(w_buf[par][p, i], BF16))
                y = y.reshape(n_seg, n_tail, Dh).astype(BF16)
                for t in range(n_part):
                    repack(src, w_buf[1 - par], p + par, i * n_part + t)
                    stage[c, pl.ds(i * n_seg + t * part, part)] = y[t * part:(t + 1) * part]
        return carry

    lax.fori_loop(0, c_wo // 2, functools.partial(pair_body, with_wo=False), 0)
    lax.fori_loop(c_wo // 2, n_ahead // 2, functools.partial(pair_body, with_wo=True), 0)
    for c in range(n_ahead + 1, n_chunk):
        w_copy(c // n_grp, c).wait()
    cp_x.wait()
    for cp in cp_ffn:
        cp.start()

    def project_tail(j, grp):
        half = UNROLL * n_tail // 2
        rows = pl.ds(grp * half if isinstance(grp, int) else pl.multiple_of(grp * half, half), half)
        y = _dot(pltpu.bitcast(xt_v[rows, :], BF16), w_tile(j))
        stage[j // HG, pl.ds((j % HG) * n_seg + grp * UNROLL, UNROLL)] = (
            y.reshape(UNROLL, n_tail, Dh).astype(BF16))

    for c in range(n_ahead, n_chunk):
        for i in range(HG):
            project_tail(c * HG + i, 0)
        if c + 1 < n_chunk:
            for t in range(n_rep):
                repack(c + 1, w_buf[(c + 1) % 2], (c + 1) // 2, t)

    acc_v[...] = jnp.zeros(acc_v.shape, F32)
    acc_v[0:M, :] = mem0_ref[...].astype(F32)
    r_at = (n_chunk, pl.ds(0, seg // HG))
    stage[r_at] = jnp.full((seg // HG, HG, LANES), -jnp.inf, BF16)

    def scores():
        return stage[r_at].astype(F32).reshape(seg, LANES)

    def norm_head(sg):
        xh_v[...] = _layernorm(x_v[sg].astype(F32)[:n_head])

    norm_head(0)

    def route(hn):
        w = wr_ref[...].astype(F32)
        w = jnp.concatenate([w[i:i + 1] for i in range(w.shape[0])], axis=1)
        return _rb(jnp.sum(hn * w, axis=-1, keepdims=True))

    early = (n_seg - UNROLL - 1) * seg
    cp_early = pltpu.make_async_copy(out_v.at[pl.ds(0, early)], out_hbm.at[pl.ds(0, early)], sem.at[4])
    cp_late = pltpu.make_async_copy(out_v.at[pl.ds(early, S - early)],
                                    out_hbm.at[pl.ds(early, S - early)], sem.at[5])

    def finish_segment(sp, lane_id):
        rows = pl.ds(pl.multiple_of(sp * seg, seg), seg)
        h = _rb(x_v[sp].astype(F32) + _rb(acc_v[M:L, :]))
        hn = _layernorm(h)
        r = route(hn)
        h_v[rows, :] = h
        out_v[rows, :] = (h + hn).astype(BF16)
        lane = lax.broadcasted_iota(jnp.int32, (seg, LANES), 1)
        r = jnp.where(lane == lane_id, r, scores())
        stage[r_at] = r.reshape(seg // HG, HG, LANES).astype(BF16)

    def step(s):
        lhs = jnp.concatenate([acc_v[0:M, :], xh_v[...]], axis=0).astype(BF16)
        norm_head(jnp.minimum(s + 1, n_seg - 1))
        qi = lax.broadcasted_iota(jnp.int32, (L, L), 0)
        ki = lax.broadcasted_iota(jnp.int32, (L, L), 1)
        visible = (qi < M) | (qi >= ki)

        def proj(m, h):
            j = m * H + h
            tail = stage[j // HG, (j % HG) * n_seg + s].astype(F32)
            return jnp.concatenate([_dot(lhs, w_tile(j)), tail], axis=0)

        val = {}
        acc = None
        for kind, h in _issue_order(H):
            if (kind, h) == ("q", H // 2):
                finish_segment(jnp.maximum(s - 1, 0), s - 1)
            if kind in "qkv":
                val[kind, h] = proj("qkv".index(kind), h)
            elif kind == "s":
                sc = _dot(val.pop(("q", h)), val.pop(("k", h)), NT) * (scale * LOG2E)
                sc = jnp.where(visible, sc, MASKED * LOG2E)
                ex = jnp.exp2(sc - jnp.max(sc, axis=-1, keepdims=True))
                val[kind, h] = ex, _recip(jnp.sum(ex, axis=-1, keepdims=True))
            elif kind == "p":
                ex, inv = val.pop(("s", h))
                val[kind, h] = _dot(ex, val.pop(("v", h))) * inv
            else:
                w = w_tile(3 * H + h)
                w = jnp.concatenate([w[t * Dh:(t + 1) * Dh] for t in range(n_col)], axis=1)
                y = _dot(val.pop(("p", h)), w)
                acc = y if acc is None else acc + y
        acc_v[...] = acc

    n_iter = n_seg // UNROLL
    late = range(n_ahead * HG, n_chunk * HG)

    def group(t, carry):
        pl.when(t == n_iter - 1)(cp_early.start)
        for u in range(UNROLL):
            step(t * UNROLL + u)
            for j in late[u::UNROLL - 1] if u < UNROLL - 1 else ():
                project_tail(j, jnp.minimum(t + 1, n_iter - 1))
        return carry

    lax.fori_loop(0, n_iter, group, 0)
    finish_segment(n_seg - 1, n_seg - 1)
    cp_late.start()

    r = scores()
    pos = (lax.broadcasted_iota(jnp.int32, r.shape, 1) * seg
           + lax.broadcasted_iota(jnp.int32, r.shape, 0))
    r = jnp.where(r != r, -jnp.inf, r)
    big = r.shape[0] * r.shape[1]
    r0 = jnp.max(r)
    i0 = jnp.min(jnp.where(r == r0, pos, big))
    rest = jnp.where(pos == i0, -jnp.inf, r)
    r1 = jnp.max(rest)
    i1 = jnp.min(jnp.where((rest == r1) & (pos != i0), pos, big))
    i0 = jnp.clip(i0, 0, S - 1)
    i1 = jnp.clip(i1, 0, S - 1)

    first = lax.broadcasted_iota(jnp.int32, (8, D), 0) == 0
    h_sel = jnp.where(first, h_v[pl.ds(i0, 1), :], h_v[pl.ds(i1, 1), :])
    hn_sel = _layernorm(h_sel)
    r_sel = route(hn_sel)
    for cp in cp_ffn:
        cp.wait()
    g = _rb(_dot(hn_sel, wg_v[...]))
    u = _rb(_dot(hn_sel, wu_v[...]))
    g = _rb(g * _rb(jax.nn.sigmoid(g)))
    y = _rb(_dot(_rb(g * u), wd_v[...]))
    y = _rb(y * _rb(jax.nn.sigmoid(r_sel)))
    new = h_sel + _rb(hn_sel + y)

    cp_early.wait()
    cp_late.wait()
    tile = 16
    fix = []
    for t, idx in enumerate((i0, i1)):
        start = pl.multiple_of((idx // tile) * tile, tile)
        rows = pl.ds(start, tile)
        hit = lax.broadcasted_iota(jnp.int32, (tile, D), 0) == idx - start
        out_v[rows, :] = jnp.where(hit, new[t:t + 1], out_v[rows, :].astype(F32)).astype(BF16)
        fix.append(pltpu.make_async_copy(out_v.at[rows], out_hbm.at[rows], sem.at[4 + t]))
    two_tiles = i0 // tile != i1 // tile
    fix[0].start()
    pl.when(two_tiles)(fix[1].start)
    fix[0].wait()
    pl.when(two_tiles)(fix[1].wait)


@functools.partial(jax.jit, static_argnames=("A_seg_len",))
def pallas_sequential_preLN__memory_aug_recurrent_mem_tr__moe_arch_mod__prompt_kernel(
    A_x: jax.Array,
    A_mem0: jax.Array,
    A_Wq: jax.Array,
    A_Wk: jax.Array,
    A_Wv: jax.Array,
    A_Wo: jax.Array,
    A_seg_len: int,
    B_x: jax.Array,
    B_w_r: jax.Array,
    B_w_gate: jax.Array,
    B_w_up: jax.Array,
    B_w_down: jax.Array,
):
    del B_x
    B, S, D = A_x.shape
    M = A_mem0.shape[1]
    _, H, Dh = A_Wq.shape
    F = B_w_gate.shape[1]
    seg = int(A_seg_len)
    n_seg = S // seg
    assert B == 1 and Dh == LANES and n_seg <= LANES and S % (2 * seg) == 0 and H % HG == 0

    hbm = pl.BlockSpec(memory_space=pl.ANY)
    vmem = pl.BlockSpec(memory_space=pltpu.VMEM)
    n_chunk = 3 * (H // HG)
    out = pl.pallas_call(
        _kernel,
        out_shape=jax.ShapeDtypeStruct((S, D), BF16),
        in_specs=[hbm, vmem, hbm, hbm, hbm, hbm, vmem, hbm, hbm, hbm],
        out_specs=hbm,
        scratch_shapes=[
            pltpu.VMEM((n_seg, seg, D), BF16),
            pltpu.VMEM((n_seg, M, D), BF16),
            pltpu.VMEM((seg - M, D), F32),
            pltpu.VMEM((n_seg * M // 2, D), U32),
            pltpu.VMEM((n_chunk + 1, D, HG, Dh), BF16),
            pltpu.VMEM((2 * H // HG, HG, D // 2, Dh), U32),
            pltpu.VMEM((2 * H // HG, HG, D // 2, Dh), U32),
            pltpu.VMEM((H, Dh, D), BF16),
            pltpu.VMEM((D, F), BF16),
            pltpu.VMEM((D, F), BF16),
            pltpu.VMEM((F, D), BF16),
            pltpu.VMEM((M + seg, D), F32),
            pltpu.VMEM((S, D), F32),
            pltpu.VMEM((S, D), BF16),
            pltpu.SemaphoreType.DMA((n_chunk,)),
            pltpu.SemaphoreType.DMA((H // HG,)),
            pltpu.SemaphoreType.DMA((7,)),
        ],
        compiler_params=pltpu.CompilerParams(vmem_limit_bytes=110 * 1024 * 1024),
        name="rmt_mod_block",
    )(
        A_x.reshape(n_seg, seg, D), A_mem0.reshape(M, D), A_Wq, A_Wk, A_Wv, A_Wo,
        B_w_r.reshape(D // LANES, LANES), B_w_gate, B_w_up, B_w_down,
    )
    return out.reshape(B, S, D)
```

```python
import functools

import jax
import jax.numpy as jnp
import numpy as np
from jax import lax
from jax.experimental import pallas as pl
from jax.experimental.pallas import tpu as pltpu

F32 = jnp.float32
BF16 = jnp.bfloat16
U32 = jnp.uint32
EPS = 1e-05
MASKED = -1000000000.0
LOG2E = 1.4426950408889634
NN = (((1,), (0,)), ((), ()))
NT = (((1,), (1,)), ((), ()))
LANES = 128
HG = 8
UNROLL = 4


def _rb(v):
    return v.astype(BF16).astype(F32)


def _layernorm(v):
    m = jnp.mean(v, axis=-1, keepdims=True)
    c = v - m
    var = jnp.mean(c * c, axis=-1, keepdims=True)
    sd = _rb(jnp.sqrt(_rb(_rb(var) + EPS)))
    return _rb(_rb(v - _rb(m)) / sd)


def _recip(v):
    r = pl.reciprocal(v, approx=True)
    return r + r * (1.0 - v * r)


def _dot(a, b, dims=NN):
    return lax.dot_general(a, b, dims, preferred_element_type=F32)


def _issue_order(n_heads):
    lag_v, lag_o = 7, 7
    cost = {"q": 32, "k": 32, "v": 32, "s": 10, "p": 10, "o": 40}
    lat_mxu, lat_softmax = 230, 480
    needs = {"s": (("k", lat_mxu),), "p": (("v", lat_mxu), ("s", lat_softmax)), "o": (("p", lat_mxu),)}
    proj = []
    for i in range(n_heads + lag_v):
        proj += [("q", i), ("k", i)] if i < n_heads else []
        proj += [("v", i - lag_v)] if i >= lag_v else []
    nxt = {"s": 0, "p": 0, "o": 0}
    done, order, now = {}, [], 0

    def ready_at(kind):
        h = nxt[kind]
        if h == n_heads or any((d, h) not in done for d, _ in needs[kind]):
            return None
        return max(done[d, h] + lat for d, lat in needs[kind])

    while len(order) < 6 * n_heads:
        at = {kind: ready_at(kind) for kind in nxt}
        if proj and ("v", min(nxt["o"] + lag_o, n_heads - 1)) not in done:
            at["o"] = None
        kinds = [kind for kind in nxt if at[kind] is not None]
        if not proj:
            now = max(now, min(at[kind] for kind in kinds))
        kinds = [kind for kind in kinds if at[kind] <= now]
        if kinds:
            op = (kinds[0], nxt[kinds[0]])
            nxt[kinds[0]] += 1
        else:
            op = proj.pop(0)
        now += cost[op[0]]
        done[op] = now
        order.append(op)
    return order


def _kernel(x_hbm, mem0_hbm, wq_hbm, wk_hbm, wv_hbm, wo_hbm, wr_hbm, wg_hbm, wu_hbm, wd_hbm,
            out_hbm,
            x_v, mem0_v, wr_v, wg_v, wu_v, wd_v, xt_raw, xh_v, xt_v, stage, w_even, w_odd, wo_raw,
            acc_v, h_v, hn_v, out_v, sem_w, sem_first, sem_wo, sem):
    n_seg, seg, D = x_v.shape
    S = n_seg * seg
    M = mem0_v.shape[0]
    H, Dh, _ = wo_raw.shape
    L = M + seg
    n_tail = xt_raw.shape[1]
    n_head = seg - n_tail
    scale = Dh ** (-0.5)
    n_grp = H // HG
    n_chunk = 3 * n_grp
    n_ahead = n_chunk - 2
    c_wo = n_ahead - n_grp
    n_col = D // LANES
    n_rep = D // 16
    w_hbm = (wq_hbm, wk_hbm, wv_hbm)

    def w_copy(m, c):
        heads = pl.ds(pl.multiple_of((c - m * n_grp) * HG, HG), HG)
        return pltpu.make_async_copy(w_hbm[m].at[:, heads, :], stage.at[c], sem_w.at[c])

    def w_wait(c):
        if isinstance(c, int):
            w_copy(c // n_grp, c).wait()
        else:
            for m in range(3):
                pl.when(c // n_grp == m)(functools.partial(lambda m: w_copy(m, c).wait(), m))

    def first_copy(t):
        rows = pl.ds(t * LANES, LANES)
        return pltpu.make_async_copy(wq_hbm.at[rows, pl.ds(0, HG), :], stage.at[0, rows],
                                     sem_first.at[t])

    def wo_copy(g):
        heads = pl.ds(g * HG, HG)
        return pltpu.make_async_copy(wo_hbm.at[heads], wo_raw.at[heads], sem_wo.at[g])

    cp_tail, cp_x, cp_mem0, cp_wr, *cp_ffn = [
        pltpu.make_async_copy(src, dst, sem.at[i])
        for i, (src, dst) in enumerate((
            (x_hbm.at[:, pl.ds(n_head, n_tail), :], xt_raw), (x_hbm, x_v), (mem0_hbm, mem0_v),
            (wr_hbm, wr_v), (wg_hbm, wg_v), (wu_hbm, wu_v), (wd_hbm, wd_v)))
    ]
    sem_out = (sem.at[7], sem.at[8])

    def request(copies):
        for cp in copies:
            cp.start(priority=1)

    cp_tail.start()
    request(first_copy(t) for t in range(n_col))
    request(w_copy(c // n_grp, c) for c in range(1, c_wo + 1))

    cp_tail.wait()
    xt = _layernorm(xt_raw[...].astype(F32).reshape(n_seg * n_tail, D))
    xt_v[...] = pltpu.bitcast(xt.astype(BF16), U32)

    w_buf = (w_even, w_odd)

    def repack(src, dst, slot, i):
        v = stage[src, pl.ds(i * 16, 16)]
        v = pltpu.bitcast(v.reshape(16 * HG, Dh), U32)
        v = jnp.swapaxes(v.reshape(8, HG, Dh), 0, 1)
        rows = pl.ds(i * 8, 8) if isinstance(i, int) else pl.ds(pl.multiple_of(i * 8, 8), 8)
        for j in range(HG // 2):
            a, b = v[j], v[HG // 2 + j]
            dst[slot, 2 * j, rows, :] = (a & 0xFFFF) | (b << 16)
            dst[slot, 2 * j + 1, rows, :] = (a >> 16) | (b & np.uint32(0xFFFF0000))

    def w_tile(j):
        c = j // HG
        return pltpu.bitcast(w_buf[c % 2][c // 2, j % HG], BF16)

    def first_body(t, carry):
        first_copy(t).wait()
        for i in range(n_rep // n_col):
            repack(0, w_even, 0, t * (n_rep // n_col) + i)
        return t

    opaque_zero = lax.fori_loop(0, n_col, first_body, 0) // n_col

    def project_chunk(p, par, heads, repack_next=True, per_head=None):
        src = jnp.minimum(2 * p + par + 1, n_ahead)
        n_part = 16
        part = n_seg // n_part
        n_slot = len(heads) * n_part - n_part // 2
        for k, i in enumerate(heads):
            y = _dot(pltpu.bitcast(xt_v[...], BF16), pltpu.bitcast(w_buf[par][p, i], BF16))
            y = y.reshape(n_seg, n_tail, Dh).astype(BF16)
            if per_head is not None:
                per_head(i)
            for t in range(n_part):
                at = k * n_part + t
                for r in range(n_rep)[at * n_rep // n_slot:(at + 1) * n_rep // n_slot]:
                    if repack_next:
                        repack(src, w_buf[1 - par], p + par, r)
                stage[2 * p + par, pl.ds(i * n_seg + t * part, part)] = y[t * part:(t + 1) * part]

    def pair_body(p, carry, *, with_wo):
        def extra(i):
            g = 2 * p - c_wo
            slot = jnp.minimum((n_chunk - c_wo) // 2 + p, 2 * n_grp - 1)
            for t in range(2):
                w = pltpu.bitcast(wo_raw[(g + t) * HG + i], U32)
                w_buf[t][slot, i] = jnp.concatenate(
                    [w[:, n * LANES:(n + 1) * LANES] for n in range(n_col)], axis=0)
                repack(n_chunk - 1, w_odd, n_chunk // 2 - 1, (g + t) * HG + i)

        for par in range(2):
            w_wait(2 * p + par + 1)
            if with_wo:
                wo_copy(2 * p + par - c_wo).wait()
        for par in range(2):
            project_chunk(p, par, range(HG),
                          per_head=extra if with_wo and par == 0 else None)
        return carry

    project_chunk(opaque_zero, 0, range(HG // 2), repack_next=False)
    w_wait(1)
    project_chunk(opaque_zero, 0, range(HG // 2, HG))
    w_wait(2)
    project_chunk(opaque_zero, 1, range(HG))
    request([w_copy(2, n_chunk - 1)])
    for c in range(c_wo + 1, n_ahead + 1):
        request([w_copy(c // n_grp, c), wo_copy(c - c_wo - 1)])
    lax.fori_loop(1, c_wo // 2, functools.partial(pair_body, with_wo=False), 0)
    w_wait(n_chunk - 1)
    request([cp_x, cp_mem0, cp_wr, *cp_ffn])
    lax.fori_loop(c_wo // 2, n_ahead // 2, functools.partial(pair_body, with_wo=True), 0)
    for cp in (cp_x, cp_mem0, cp_wr):
        cp.wait()

    def project_tail(j, grp):
        half = UNROLL * n_tail // 2
        rows = pl.ds(grp * half if isinstance(grp, int) else pl.multiple_of(grp * half, half), half)
        y = _dot(pltpu.bitcast(xt_v[rows, :], BF16), w_tile(j))
        stage[j // HG, pl.ds((j % HG) * n_seg + grp * UNROLL, UNROLL)] = (
            y.reshape(UNROLL, n_tail, Dh).astype(BF16))

    late = range(n_ahead * HG, n_chunk * HG)
    for j in late:
        project_tail(j, 0)

    acc_v[...] = jnp.zeros(acc_v.shape, F32)
    acc_v[0:M, :] = mem0_v[...].astype(F32)
    r_at = (n_chunk, pl.ds(0, seg // HG))
    stage[r_at] = jnp.full((seg // HG, HG, LANES), -jnp.inf, BF16)

    def scores():
        return stage[r_at].astype(F32).reshape(seg, LANES)

    def norm_head(sg):
        xh_v[...] = _layernorm(x_v[sg].astype(F32)[:n_head])

    norm_head(0)

    def route(hn):
        w = wr_v[...].astype(F32)
        w = jnp.concatenate([w[i:i + 1] for i in range(w.shape[0])], axis=1)
        return _rb(jnp.sum(hn * w, axis=-1, keepdims=True))

    early = (n_seg - UNROLL - 1) * seg
    cp_early = pltpu.make_async_copy(out_v.at[pl.ds(0, early)], out_hbm.at[pl.ds(0, early)], sem_out[0])
    cp_late = pltpu.make_async_copy(out_v.at[pl.ds(early, S - early)],
                                    out_hbm.at[pl.ds(early, S - early)], sem_out[1])

    def finish_segment(sp, lane_id):
        rows = pl.ds(pl.multiple_of(sp * seg, seg), seg)
        h = _rb(x_v[sp].astype(F32) + _rb(acc_v[M:L, :]))
        hn = _layernorm(h)
        r = route(hn)
        h_v[rows, :] = h
        hn_v[rows, :] = hn
        out_v[rows, :] = (h + hn).astype(BF16)
        lane = lax.broadcasted_iota(jnp.int32, (seg, LANES), 1)
        r = jnp.where(lane == lane_id, r, scores())
        stage[r_at] = r.reshape(seg // HG, HG, LANES).astype(BF16)

    def step(s):
        lhs = jnp.concatenate([acc_v[0:M, :], xh_v[...]], axis=0).astype(BF16)
        norm_head(jnp.minimum(s + 1, n_seg - 1))
        qi = lax.broadcasted_iota(jnp.int32, (L, L), 0)
        ki = lax.broadcasted_iota(jnp.int32, (L, L), 1)
        visible = (qi < M) | (qi >= ki)

        def proj(m, h):
            j = m * H + h
            tail = stage[j // HG, (j % HG) * n_seg + s].astype(F32)
            return jnp.concatenate([_dot(lhs, w_tile(j)), tail], axis=0)

        val = {}
        acc = None
        for kind, h in _issue_order(H):
            if (kind, h) == ("q", H // 2):
                finish_segment(jnp.maximum(s - 1, 0), s - 1)
            if kind in "qkv":
                val[kind, h] = proj("qkv".index(kind), h)
            elif kind == "s":
                sc = _dot(val.pop(("q", h)), val.pop(("k", h)), NT) * (scale * LOG2E)
                sc = jnp.where(visible, sc, MASKED * LOG2E)
                ex = jnp.exp2(sc - jnp.max(sc, axis=-1, keepdims=True))
                val[kind, h] = ex, _recip(jnp.sum(ex, axis=-1, keepdims=True))
            elif kind == "p":
                ex, inv = val.pop(("s", h))
                val[kind, h] = _dot(ex, val.pop(("v", h))) * inv
            else:
                w = w_tile(3 * H + h)
                w = jnp.concatenate([w[t * Dh:(t + 1) * Dh] for t in range(n_col)], axis=1)
                y = _dot(val.pop(("p", h)), w)
                acc = y if acc is None else acc + y
        acc_v[...] = acc

    n_iter = n_seg // UNROLL

    def group(t, carry):
        pl.when(t == n_iter - 1)(cp_early.start)
        for u in range(UNROLL):
            step(t * UNROLL + u)
            for j in late[u::UNROLL - 1] if u < UNROLL - 1 else ():
                project_tail(j, jnp.minimum(t + 1, n_iter - 1))
        return carry

    lax.fori_loop(0, n_iter, group, 0)
    for cp in cp_ffn:
        cp.wait()
    finish_segment(n_seg - 1, n_seg - 1)
    cp_late.start()

    r = scores()
    pos = (lax.broadcasted_iota(jnp.int32, r.shape, 1) * seg
           + lax.broadcasted_iota(jnp.int32, r.shape, 0))
    r = jnp.where(r != r, -jnp.inf, r)
    big = r.shape[0] * r.shape[1]
    r0 = jnp.max(r)
    i0 = jnp.min(jnp.where(r == r0, pos, big))
    rest = jnp.where(pos == i0, -jnp.inf, r)
    r1 = jnp.max(rest)
    i1 = jnp.min(jnp.where((rest == r1) & (pos != i0), pos, big))
    i0 = jnp.clip(i0, 0, S - 1)
    i1 = jnp.clip(i1, 0, S - 1)

    first = lax.broadcasted_iota(jnp.int32, (8, D), 0) == 0
    h_sel = jnp.where(first, h_v[pl.ds(i0, 1), :], h_v[pl.ds(i1, 1), :])
    hn_sel = jnp.where(first, hn_v[pl.ds(i0, 1), :], hn_v[pl.ds(i1, 1), :])
    r_sel = route(hn_sel)
    g = _rb(_dot(hn_sel, wg_v[...]))
    u = _rb(_dot(hn_sel, wu_v[...]))
    g = _rb(g * _rb(jax.nn.sigmoid(g)))
    y = _rb(_dot(_rb(g * u), wd_v[...]))
    y = _rb(y * _rb(jax.nn.sigmoid(r_sel)))
    new = h_sel + _rb(hn_sel + y)

    cp_early.wait()
    cp_late.wait()
    tile = 16
    fix = []
    for t, idx in enumerate((i0, i1)):
        start = pl.multiple_of((idx // tile) * tile, tile)
        rows = pl.ds(start, tile)
        hit = lax.broadcasted_iota(jnp.int32, (tile, D), 0) == idx - start
        out_v[rows, :] = jnp.where(hit, new[t:t + 1], out_v[rows, :].astype(F32)).astype(BF16)
        fix.append(pltpu.make_async_copy(out_v.at[rows], out_hbm.at[rows], sem_out[t]))
    two_tiles = i0 // tile != i1 // tile
    fix[0].start()
    pl.when(two_tiles)(fix[1].start)
    fix[0].wait()
    pl.when(two_tiles)(fix[1].wait)


@functools.partial(jax.jit, static_argnames=("A_seg_len",))
def pallas_sequential_preLN__memory_aug_recurrent_mem_tr__moe_arch_mod__prompt_kernel(
    A_x: jax.Array,
    A_mem0: jax.Array,
    A_Wq: jax.Array,
    A_Wk: jax.Array,
    A_Wv: jax.Array,
    A_Wo: jax.Array,
    A_seg_len: int,
    B_x: jax.Array,
    B_w_r: jax.Array,
    B_w_gate: jax.Array,
    B_w_up: jax.Array,
    B_w_down: jax.Array,
):
    del B_x
    B, S, D = A_x.shape
    M = A_mem0.shape[1]
    _, H, Dh = A_Wq.shape
    F = B_w_gate.shape[1]
    seg = int(A_seg_len)
    n_seg = S // seg
    assert B == 1 and Dh == LANES and n_seg <= LANES and S % (2 * seg) == 0 and H % HG == 0

    hbm = pl.BlockSpec(memory_space=pl.ANY)
    n_chunk = 3 * (H // HG)
    out = pl.pallas_call(
        _kernel,
        out_shape=jax.ShapeDtypeStruct((S, D), BF16),
        in_specs=[hbm] * 10,
        out_specs=hbm,
        scratch_shapes=[
            pltpu.VMEM((n_seg, seg, D), BF16),
            pltpu.VMEM((M, D), BF16),
            pltpu.VMEM((D // LANES, LANES), BF16),
            pltpu.VMEM((D, F), BF16),
            pltpu.VMEM((D, F), BF16),
            pltpu.VMEM((F, D), BF16),
            pltpu.VMEM((n_seg, M, D), BF16),
            pltpu.VMEM((seg - M, D), F32),
            pltpu.VMEM((n_seg * M // 2, D), U32),
            pltpu.VMEM((n_chunk + 1, D, HG, Dh), BF16),
            pltpu.VMEM((2 * H // HG, HG, D // 2, Dh), U32),
            pltpu.VMEM((2 * H // HG, HG, D // 2, Dh), U32),
            pltpu.VMEM((H, Dh, D), BF16),
            pltpu.VMEM((M + seg, D), F32),
            pltpu.VMEM((S, D), F32),
            pltpu.VMEM((S, D), F32),
            pltpu.VMEM((S, D), BF16),
            pltpu.SemaphoreType.DMA((n_chunk,)),
            pltpu.SemaphoreType.DMA((D // LANES,)),
            pltpu.SemaphoreType.DMA((H // HG,)),
            pltpu.SemaphoreType.DMA((9,)),
        ],
        compiler_params=pltpu.CompilerParams(vmem_limit_bytes=110 * 1024 * 1024),
        name="rmt_mod_block",
    )(
        A_x.reshape(n_seg, seg, D), A_mem0.reshape(M, D), A_Wq, A_Wk, A_Wv, A_Wo,
        B_w_r.reshape(D // LANES, LANES), B_w_gate, B_w_up, B_w_down,
    )
    return out.reshape(B, S, D)
```

```python
import functools

import jax
import jax.numpy as jnp
import numpy as np
from jax import lax
from jax.experimental import pallas as pl
from jax.experimental.pallas import tpu as pltpu

F32 = jnp.float32
BF16 = jnp.bfloat16
U32 = jnp.uint32
EPS = 1e-05
MASKED = -1000000000.0
LOG2E = 1.4426950408889634
NN = (((1,), (0,)), ((), ()))
NT = (((1,), (1,)), ((), ()))
LANES = 128
HG = 8
UNROLL = 4


def _rb(v):
    return v.astype(BF16).astype(F32)


def _layernorm(v):
    m = jnp.mean(v, axis=-1, keepdims=True)
    c = v - m
    var = jnp.mean(c * c, axis=-1, keepdims=True)
    sd = _rb(jnp.sqrt(_rb(_rb(var) + EPS)))
    return _rb(_rb(v - _rb(m)) / sd)


def _recip(v):
    r = pl.reciprocal(v, approx=True)
    return r + r * (1.0 - v * r)


def _dot(a, b, dims=NN):
    return lax.dot_general(a, b, dims, preferred_element_type=F32)


def _issue_order(n_heads):
    lag_v, lag_o = 7, 7
    cost = {"q": 32, "k": 32, "v": 32, "s": 10, "p": 10, "o": 40}
    lat_mxu, lat_softmax = 230, 480
    needs = {"s": (("k", lat_mxu),), "p": (("v", lat_mxu), ("s", lat_softmax)), "o": (("p", lat_mxu),)}
    proj = []
    for i in range(n_heads + lag_v):
        proj += [("q", i), ("k", i)] if i < n_heads else []
        proj += [("v", i - lag_v)] if i >= lag_v else []
    nxt = {"s": 0, "p": 0, "o": 0}
    done, order, now = {}, [], 0

    def ready_at(kind):
        h = nxt[kind]
        if h == n_heads or any((d, h) not in done for d, _ in needs[kind]):
            return None
        return max(done[d, h] + lat for d, lat in needs[kind])

    while len(order) < 6 * n_heads:
        at = {kind: ready_at(kind) for kind in nxt}
        if proj and ("v", min(nxt["o"] + lag_o, n_heads - 1)) not in done:
            at["o"] = None
        kinds = [kind for kind in nxt if at[kind] is not None]
        if not proj:
            now = max(now, min(at[kind] for kind in kinds))
        kinds = [kind for kind in kinds if at[kind] <= now]
        if kinds:
            op = (kinds[0], nxt[kinds[0]])
            nxt[kinds[0]] += 1
        else:
            op = proj.pop(0)
        now += cost[op[0]]
        done[op] = now
        order.append(op)
    return order


def _kernel(x_hbm, mem0_hbm, wq_hbm, wk_hbm, wv_hbm, wo_hbm, wr_hbm, wg_hbm, wu_hbm, wd_hbm,
            out_hbm,
            x_v, mem0_v, wr_v, wg_v, wu_v, wd_v, xt_raw, xh_v, xt_v, stage, w_even, w_odd, wo_raw,
            acc_v, h_v, hn_v, out_v, sem_w, sem_first, sem_wo, sem):
    n_seg, seg, D = x_v.shape
    S = n_seg * seg
    M = mem0_v.shape[0]
    H, Dh, _ = wo_raw.shape
    L = M + seg
    n_tail = xt_raw.shape[1]
    n_head = seg - n_tail
    scale = Dh ** (-0.5)
    n_grp = H // HG
    n_chunk = 3 * n_grp
    n_ahead = n_chunk - 2
    c_wo = n_ahead - n_grp
    n_col = D // LANES
    n_rep = D // 16
    w_hbm = (wq_hbm, wk_hbm, wv_hbm)

    def w_copy(m, c):
        heads = pl.ds(pl.multiple_of((c - m * n_grp) * HG, HG), HG)
        return pltpu.make_async_copy(w_hbm[m].at[:, heads, :], stage.at[c], sem_w.at[c])

    def w_wait(c):
        if isinstance(c, int):
            w_copy(c // n_grp, c).wait()
        else:
            for m in range(3):
                pl.when(c // n_grp == m)(functools.partial(lambda m: w_copy(m, c).wait(), m))

    def first_copy(t):
        rows = pl.ds(t * LANES, LANES)
        return pltpu.make_async_copy(wq_hbm.at[rows, pl.ds(0, HG), :], stage.at[0, rows],
                                     sem_first.at[t])

    def wo_copy(g):
        heads = pl.ds(g * HG, HG)
        return pltpu.make_async_copy(wo_hbm.at[heads], wo_raw.at[heads], sem_wo.at[g])

    cp_tail, cp_x, cp_mem0, cp_wr, *cp_ffn = [
        pltpu.make_async_copy(src, dst, sem.at[i])
        for i, (src, dst) in enumerate((
            (x_hbm.at[:, pl.ds(n_head, n_tail), :], xt_raw), (x_hbm, x_v), (mem0_hbm, mem0_v),
            (wr_hbm, wr_v), (wg_hbm, wg_v), (wu_hbm, wu_v), (wd_hbm, wd_v)))
    ]
    sem_out = (sem.at[7], sem.at[8])

    def request(copies):
        for cp in copies:
            cp.start(priority=1)

    cp_tail.start()
    request(first_copy(t) for t in range(n_col))
    request(w_copy(c // n_grp, c) for c in range(1, c_wo + 1))

    cp_tail.wait()
    xt = _layernorm(xt_raw[...].astype(F32).reshape(n_seg * n_tail, D))
    xt_v[...] = pltpu.bitcast(xt.astype(BF16), U32)

    w_buf = (w_even, w_odd)

    def repack(src, dst, slot, i):
        v = stage[src, pl.ds(i * 16, 16)]
        v = pltpu.bitcast(v.reshape(16 * HG, Dh), U32)
        v = jnp.swapaxes(v.reshape(8, HG, Dh), 0, 1)
        rows = pl.ds(i * 8, 8) if isinstance(i, int) else pl.ds(pl.multiple_of(i * 8, 8), 8)
        for j in range(HG // 2):
            a, b = v[j], v[HG // 2 + j]
            dst[slot, 2 * j, rows, :] = (a & 0xFFFF) | (b << 16)
            dst[slot, 2 * j + 1, rows, :] = (a >> 16) | (b & np.uint32(0xFFFF0000))

    def w_tile(j):
        c = j // HG
        return pltpu.bitcast(w_buf[c % 2][c // 2, j % HG], BF16)

    def first_body(t, carry):
        first_copy(t).wait()
        for i in range(n_rep // n_col):
            repack(0, w_even, 0, t * (n_rep // n_col) + i)
        return t

    opaque_zero = lax.fori_loop(0, n_col, first_body, 0) // n_col

    def project_chunk(p, par, heads, repack_next=True, per_head=None):
        src = jnp.minimum(2 * p + par + 1, n_ahead)
        n_part = 16
        part = n_seg // n_part
        n_slot = len(heads) * n_part - n_part // 2
        for k, i in enumerate(heads):
            y = _dot(pltpu.bitcast(xt_v[...], BF16), pltpu.bitcast(w_buf[par][p, i], BF16))
            y = y.reshape(n_seg, n_tail, Dh).astype(BF16)
            if per_head is not None:
                per_head(i)
            for t in range(n_part):
                at = k * n_part + t
                for r in range(n_rep)[at * n_rep // n_slot:(at + 1) * n_rep // n_slot]:
                    if repack_next:
                        repack(src, w_buf[1 - par], p + par, r)
                stage[2 * p + par, pl.ds(i * n_seg + t * part, part)] = y[t * part:(t + 1) * part]

    def pair_body(p, carry, *, with_wo):
        def extra(i):
            g = 2 * p - c_wo
            slot = jnp.minimum((n_chunk - c_wo) // 2 + p, 2 * n_grp - 1)
            for t in range(2):
                w = pltpu.bitcast(wo_raw[(g + t) * HG + i], U32)
                w_buf[t][slot, i] = jnp.concatenate(
                    [w[:, n * LANES:(n + 1) * LANES] for n in range(n_col)], axis=0)
                repack(n_chunk - 1, w_odd, n_chunk // 2 - 1, (g + t) * HG + i)

        for par in range(2):
            w_wait(2 * p + par + 1)
            if with_wo:
                wo_copy(2 * p + par - c_wo).wait()
        for par in range(2):
            project_chunk(p, par, range(HG),
                          per_head=extra if with_wo and par == 0 else None)
        return carry

    def request_with_wo(chunks):
        for c in chunks:
            request([w_copy(c // n_grp, c), wo_copy(c - c_wo - 1)])

    project_chunk(opaque_zero, 0, range(HG // 2), repack_next=False)
    request([w_copy(2, n_chunk - 1)])
    request_with_wo(range(c_wo + 1, c_wo + 3))
    w_wait(1)
    project_chunk(opaque_zero, 0, range(HG // 2, HG))
    w_wait(2)
    project_chunk(opaque_zero, 1, range(HG))
    request_with_wo(range(c_wo + 3, n_ahead + 1))
    lax.fori_loop(1, c_wo // 2, functools.partial(pair_body, with_wo=False), 0)
    w_wait(n_chunk - 1)
    request([cp_x, cp_mem0, cp_wr, *cp_ffn])
    lax.fori_loop(c_wo // 2, n_ahead // 2, functools.partial(pair_body, with_wo=True), 0)
    for cp in (cp_x, cp_mem0, cp_wr):
        cp.wait()

    def project_tail(j, grp):
        half = UNROLL * n_tail // 2
        rows = pl.ds(grp * half if isinstance(grp, int) else pl.multiple_of(grp * half, half), half)
        y = _dot(pltpu.bitcast(xt_v[rows, :], BF16), w_tile(j))
        stage[j // HG, pl.ds((j % HG) * n_seg + grp * UNROLL, UNROLL)] = (
            y.reshape(UNROLL, n_tail, Dh).astype(BF16))

    late = range(n_ahead * HG, n_chunk * HG)
    for j in late:
        project_tail(j, 0)

    acc_v[...] = jnp.zeros(acc_v.shape, F32)
    acc_v[0:M, :] = mem0_v[...].astype(F32)
    r_at = (n_chunk, pl.ds(0, seg // HG))
    stage[r_at] = jnp.full((seg // HG, HG, LANES), -jnp.inf, BF16)

    def scores():
        return stage[r_at].astype(F32).reshape(seg, LANES)

    def norm_head(sg):
        xh_v[...] = _layernorm(x_v[sg].astype(F32)[:n_head])

    norm_head(0)

    def route(hn):
        w = wr_v[...].astype(F32)
        w = jnp.concatenate([w[i:i + 1] for i in range(w.shape[0])], axis=1)
        return _rb(jnp.sum(hn * w, axis=-1, keepdims=True))

    early = (n_seg - UNROLL - 1) * seg
    cp_early = pltpu.make_async_copy(out_v.at[pl.ds(0, early)], out_hbm.at[pl.ds(0, early)], sem_out[0])
    cp_late = pltpu.make_async_copy(out_v.at[pl.ds(early, S - early)],
                                    out_hbm.at[pl.ds(early, S - early)], sem_out[1])

    def finish_segment(sp, lane_id):
        rows = pl.ds(pl.multiple_of(sp * seg, seg), seg)
        h = _rb(x_v[sp].astype(F32) + _rb(acc_v[M:L, :]))
        hn = _layernorm(h)
        r = route(hn)
        h_v[rows, :] = h
        hn_v[rows, :] = hn
        out_v[rows, :] = (h + hn).astype(BF16)
        lane = lax.broadcasted_iota(jnp.int32, (seg, LANES), 1)
        r = jnp.where(lane == lane_id, r, scores())
        stage[r_at] = r.reshape(seg // HG, HG, LANES).astype(BF16)

    def step(s):
        lhs = jnp.concatenate([acc_v[0:M, :], xh_v[...]], axis=0).astype(BF16)
        norm_head(jnp.minimum(s + 1, n_seg - 1))
        qi = lax.broadcasted_iota(jnp.int32, (L, L), 0)
        ki = lax.broadcasted_iota(jnp.int32, (L, L), 1)
        visible = (qi < M) | (qi >= ki)

        def proj(m, h):
            j = m * H + h
            tail = stage[j // HG, (j % HG) * n_seg + s].astype(F32)
            return jnp.concatenate([_dot(lhs, w_tile(j)), tail], axis=0)

        val = {}
        acc = None
        for kind, h in _issue_order(H):
            if (kind, h) == ("q", 8):
                finish_segment(jnp.maximum(s - 1, 0), s - 1)
            if kind in "qkv":
                val[kind, h] = proj("qkv".index(kind), h)
            elif kind == "s":
                sc = _dot(val.pop(("q", h)), val.pop(("k", h)), NT) * (scale * LOG2E)
                sc = jnp.where(visible, sc, MASKED * LOG2E)
                ex = jnp.exp2(sc - jnp.max(sc, axis=-1, keepdims=True))
                val[kind, h] = ex, _recip(jnp.sum(ex, axis=-1, keepdims=True))
            elif kind == "p":
                ex, inv = val.pop(("s", h))
                val[kind, h] = _dot(ex, val.pop(("v", h))) * inv
            else:
                w = w_tile(3 * H + h)
                w = jnp.concatenate([w[t * Dh:(t + 1) * Dh] for t in range(n_col)], axis=1)
                y = _dot(val.pop(("p", h)), w)
                acc = y if acc is None else acc + y
        acc_v[...] = acc

    n_iter = n_seg // UNROLL

    def group(t, carry):
        pl.when(t == n_iter - 1)(cp_early.start)
        for u in range(UNROLL):
            step(t * UNROLL + u)
            for j in late[u::UNROLL - 1] if u < UNROLL - 1 else ():
                project_tail(j, jnp.minimum(t + 1, n_iter - 1))
        return carry

    lax.fori_loop(0, n_iter, group, 0)
    for cp in cp_ffn:
        cp.wait()
    finish_segment(n_seg - 1, n_seg - 1)
    cp_late.start()

    r = scores()
    pos = (lax.broadcasted_iota(jnp.int32, r.shape, 1) * seg
           + lax.broadcasted_iota(jnp.int32, r.shape, 0))
    r = jnp.where(r != r, -jnp.inf, r)
    big = r.shape[0] * r.shape[1]
    r0 = jnp.max(r)
    i0 = jnp.min(jnp.where(r == r0, pos, big))
    rest = jnp.where(pos == i0, -jnp.inf, r)
    r1 = jnp.max(rest)
    i1 = jnp.min(jnp.where((rest == r1) & (pos != i0), pos, big))
    i0 = jnp.clip(i0, 0, S - 1)
    i1 = jnp.clip(i1, 0, S - 1)

    first = lax.broadcasted_iota(jnp.int32, (8, D), 0) == 0
    h_sel = jnp.where(first, h_v[pl.ds(i0, 1), :], h_v[pl.ds(i1, 1), :])
    hn_sel = jnp.where(first, hn_v[pl.ds(i0, 1), :], hn_v[pl.ds(i1, 1), :])
    r_sel = route(hn_sel)
    g = _rb(_dot(hn_sel, wg_v[...]))
    u = _rb(_dot(hn_sel, wu_v[...]))
    g = _rb(g * _rb(jax.nn.sigmoid(g)))
    y = _rb(_dot(_rb(g * u), wd_v[...]))
    y = _rb(y * _rb(jax.nn.sigmoid(r_sel)))
    new = h_sel + _rb(hn_sel + y)

    cp_early.wait()
    cp_late.wait()
    tile = 16
    fix = []
    for t, idx in enumerate((i0, i1)):
        start = pl.multiple_of((idx // tile) * tile, tile)
        rows = pl.ds(start, tile)
        hit = lax.broadcasted_iota(jnp.int32, (tile, D), 0) == idx - start
        out_v[rows, :] = jnp.where(hit, new[t:t + 1], out_v[rows, :].astype(F32)).astype(BF16)
        fix.append(pltpu.make_async_copy(out_v.at[rows], out_hbm.at[rows], sem_out[t]))
    two_tiles = i0 // tile != i1 // tile
    fix[0].start()
    pl.when(two_tiles)(fix[1].start)
    fix[0].wait()
    pl.when(two_tiles)(fix[1].wait)


@functools.partial(jax.jit, static_argnames=("A_seg_len",))
def pallas_sequential_preLN__memory_aug_recurrent_mem_tr__moe_arch_mod__prompt_kernel(
    A_x: jax.Array,
    A_mem0: jax.Array,
    A_Wq: jax.Array,
    A_Wk: jax.Array,
    A_Wv: jax.Array,
    A_Wo: jax.Array,
    A_seg_len: int,
    B_x: jax.Array,
    B_w_r: jax.Array,
    B_w_gate: jax.Array,
    B_w_up: jax.Array,
    B_w_down: jax.Array,
):
    del B_x
    B, S, D = A_x.shape
    M = A_mem0.shape[1]
    _, H, Dh = A_Wq.shape
    F = B_w_gate.shape[1]
    seg = int(A_seg_len)
    n_seg = S // seg
    assert B == 1 and Dh == LANES and n_seg <= LANES and S % (2 * seg) == 0 and H % HG == 0

    hbm = pl.BlockSpec(memory_space=pl.ANY)
    n_chunk = 3 * (H // HG)
    out = pl.pallas_call(
        _kernel,
        out_shape=jax.ShapeDtypeStruct((S, D), BF16),
        in_specs=[hbm] * 10,
        out_specs=hbm,
        scratch_shapes=[
            pltpu.VMEM((n_seg, seg, D), BF16),
            pltpu.VMEM((M, D), BF16),
            pltpu.VMEM((D // LANES, LANES), BF16),
            pltpu.VMEM((D, F), BF16),
            pltpu.VMEM((D, F), BF16),
            pltpu.VMEM((F, D), BF16),
            pltpu.VMEM((n_seg, M, D), BF16),
            pltpu.VMEM((seg - M, D), F32),
            pltpu.VMEM((n_seg * M // 2, D), U32),
            pltpu.VMEM((n_chunk + 1, D, HG, Dh), BF16),
            pltpu.VMEM((2 * H // HG, HG, D // 2, Dh), U32),
            pltpu.VMEM((2 * H // HG, HG, D // 2, Dh), U32),
            pltpu.VMEM((H, Dh, D), BF16),
            pltpu.VMEM((M + seg, D), F32),
            pltpu.VMEM((S, D), F32),
            pltpu.VMEM((S, D), F32),
            pltpu.VMEM((S, D), BF16),
            pltpu.SemaphoreType.DMA((n_chunk,)),
            pltpu.SemaphoreType.DMA((D // LANES,)),
            pltpu.SemaphoreType.DMA((H // HG,)),
            pltpu.SemaphoreType.DMA((9,)),
        ],
        compiler_params=pltpu.CompilerParams(vmem_limit_bytes=110 * 1024 * 1024),
        name="rmt_mod_block",
    )(
        A_x.reshape(n_seg, seg, D), A_mem0.reshape(M, D), A_Wq, A_Wk, A_Wv, A_Wo,
        B_w_r.reshape(D // LANES, LANES), B_w_gate, B_w_up, B_w_down,
    )
    return out.reshape(B, S, D)
```

```python
import functools

import jax
import jax.numpy as jnp
import numpy as np
from jax import lax
from jax.experimental import pallas as pl
from jax.experimental.pallas import tpu as pltpu

F32 = jnp.float32
BF16 = jnp.bfloat16
U32 = jnp.uint32
EPS = 1e-05
MASKED = -1000000000.0
LOG2E = 1.4426950408889634
NN = (((1,), (0,)), ((), ()))
NT = (((1,), (1,)), ((), ()))
LANES = 128
HG = 8
UNROLL = 8
GROUP = 4


def _rb(v):
    return v.astype(BF16).astype(F32)


def _layernorm(v):
    m = jnp.mean(v, axis=-1, keepdims=True)
    c = v - m
    var = jnp.mean(c * c, axis=-1, keepdims=True)
    sd = _rb(jnp.sqrt(_rb(_rb(var) + EPS)))
    return _rb(_rb(v - _rb(m)) / sd)


def _recip(v):
    r = pl.reciprocal(v, approx=True)
    return r + r * (1.0 - v * r)


def _dot(a, b, dims=NN):
    return lax.dot_general(a, b, dims, preferred_element_type=F32)


def _issue_order(n_heads):
    lag_v, lag_o = 7, 7
    cost = {"q": 32, "k": 32, "v": 32, "s": 10, "p": 10, "o": 40}
    lat_mxu, lat_softmax = 230, 480
    needs = {"s": (("k", lat_mxu),), "p": (("v", lat_mxu), ("s", lat_softmax)), "o": (("p", lat_mxu),)}
    proj = []
    for i in range(n_heads + lag_v):
        proj += [("q", i), ("k", i)] if i < n_heads else []
        proj += [("v", i - lag_v)] if i >= lag_v else []
    nxt = {"s": 0, "p": 0, "o": 0}
    done, order, now = {}, [], 0

    def ready_at(kind):
        h = nxt[kind]
        if h == n_heads or any((d, h) not in done for d, _ in needs[kind]):
            return None
        return max(done[d, h] + lat for d, lat in needs[kind])

    while len(order) < 6 * n_heads:
        at = {kind: ready_at(kind) for kind in nxt}
        if proj and ("v", min(nxt["o"] + lag_o, n_heads - 1)) not in done:
            at["o"] = None
        kinds = [kind for kind in nxt if at[kind] is not None]
        if not proj:
            now = max(now, min(at[kind] for kind in kinds))
        kinds = [kind for kind in kinds if at[kind] <= now]
        if kinds:
            op = (kinds[0], nxt[kinds[0]])
            nxt[kinds[0]] += 1
        else:
            op = proj.pop(0)
        now += cost[op[0]]
        done[op] = now
        order.append(op)
    return order


def _kernel(x_hbm, mem0_hbm, wq_hbm, wk_hbm, wv_hbm, wo_hbm, wr_hbm, wg_hbm, wu_hbm, wd_hbm,
            out_hbm,
            x_v, mem0_v, wr_v, wg_v, wu_v, wd_v, xt_raw, xh_v, xt_v, stage, w_even, w_odd, wo_raw,
            acc_v, h_v, hn_v, out_v, sem_w, sem_first, sem_wo, sem):
    n_seg, seg, D = x_v.shape
    S = n_seg * seg
    M = mem0_v.shape[0]
    H, Dh, _ = wo_raw.shape
    L = M + seg
    n_tail = xt_raw.shape[1]
    n_head = seg - n_tail
    scale = Dh ** (-0.5)
    n_grp = H // HG
    n_chunk = 3 * n_grp
    n_ahead = n_chunk - 2
    c_wo = n_ahead - n_grp
    n_col = D // LANES
    n_rep = D // 16
    w_hbm = (wq_hbm, wk_hbm, wv_hbm)

    def w_copy(m, c):
        heads = pl.ds(pl.multiple_of((c - m * n_grp) * HG, HG), HG)
        return pltpu.make_async_copy(w_hbm[m].at[:, heads, :], stage.at[c], sem_w.at[c])

    def w_wait(c):
        if isinstance(c, int):
            w_copy(c // n_grp, c).wait()
        else:
            for m in range(3):
                pl.when(c // n_grp == m)(functools.partial(lambda m: w_copy(m, c).wait(), m))

    def first_copy(t):
        rows = pl.ds(t * LANES, LANES)
        return pltpu.make_async_copy(wq_hbm.at[rows, pl.ds(0, HG), :], stage.at[0, rows],
                                     sem_first.at[t])

    def wo_copy(g):
        heads = pl.ds(g * HG, HG)
        return pltpu.make_async_copy(wo_hbm.at[heads], wo_raw.at[heads], sem_wo.at[g])

    cp_tail, cp_x, cp_mem0, cp_wr, *cp_ffn = [
        pltpu.make_async_copy(src, dst, sem.at[i])
        for i, (src, dst) in enumerate((
            (x_hbm.at[:, pl.ds(n_head, n_tail), :], xt_raw), (x_hbm, x_v), (mem0_hbm, mem0_v),
            (wr_hbm, wr_v), (wg_hbm, wg_v), (wu_hbm, wu_v), (wd_hbm, wd_v)))
    ]
    sem_out = (sem.at[7], sem.at[8])

    def request(copies):
        for cp in copies:
            cp.start(priority=1)

    cp_tail.start()
    request(first_copy(t) for t in range(n_col))
    request(w_copy(c // n_grp, c) for c in range(1, c_wo + 1))

    cp_tail.wait()
    xt = _layernorm(xt_raw[...].astype(F32).reshape(n_seg * n_tail, D))
    xt_v[...] = pltpu.bitcast(xt.astype(BF16), U32)

    w_buf = (w_even, w_odd)

    def repack(src, dst, slot, i):
        v = stage[src, pl.ds(i * 16, 16)]
        v = pltpu.bitcast(v.reshape(16 * HG, Dh), U32)
        v = jnp.swapaxes(v.reshape(8, HG, Dh), 0, 1)
        rows = pl.ds(i * 8, 8) if isinstance(i, int) else pl.ds(pl.multiple_of(i * 8, 8), 8)
        for j in range(HG // 2):
            a, b = v[j], v[HG // 2 + j]
            dst[slot, 2 * j, rows, :] = (a & 0xFFFF) | (b << 16)
            dst[slot, 2 * j + 1, rows, :] = (a >> 16) | (b & np.uint32(0xFFFF0000))

    def w_tile(j):
        c = j // HG
        return pltpu.bitcast(w_buf[c % 2][c // 2, j % HG], BF16)

    def first_body(t, carry):
        first_copy(t).wait()
        for i in range(n_rep // n_col):
            repack(0, w_even, 0, t * (n_rep // n_col) + i)
        return t

    opaque_zero = lax.fori_loop(0, n_col, first_body, 0) // n_col

    def project_chunk(p, par, n_heads=HG, head0=0, n_piece=n_rep, piece0=0, per_head=None):
        src = jnp.minimum(2 * p + par + 1, n_ahead)
        n_part = 16
        part = n_seg // n_part
        n_slot = n_heads * n_part - n_part // 2
        for k in range(n_heads):
            i = head0 + k
            y = _dot(pltpu.bitcast(xt_v[...], BF16), pltpu.bitcast(w_buf[par][p, i], BF16))
            y = y.reshape(n_seg, n_tail, Dh).astype(BF16)
            if per_head is not None:
                per_head(i)
            for t in range(n_part):
                at = k * n_part + t
                for r in range(n_piece)[at * n_piece // n_slot:(at + 1) * n_piece // n_slot]:
                    repack(src, w_buf[1 - par], p + par, piece0 + r)
                stage[2 * p + par, pl.ds(i * n_seg + t * part, part)] = y[t * part:(t + 1) * part]

    def pair_body(p, carry, *, with_wo):
        def extra(i):
            g = 2 * p - c_wo
            slot = jnp.minimum((n_chunk - c_wo) // 2 + p, 2 * n_grp - 1)
            for t in range(2):
                w = pltpu.bitcast(wo_raw[(g + t) * HG + i], U32)
                w_buf[t][slot, i] = jnp.concatenate(
                    [w[:, n * LANES:(n + 1) * LANES] for n in range(n_col)], axis=0)
                repack(n_chunk - 1, w_odd, n_chunk // 2 - 1, (g + t) * HG + i)

        for par in range(2):
            w_wait(2 * p + par + 1)
            if with_wo:
                wo_copy(2 * p + par - c_wo).wait()
        for par in range(2):
            project_chunk(p, par, per_head=extra if with_wo and par == 0 else None)
        return carry

    def request_with_wo(chunks):
        for c in chunks:
            request([w_copy(c // n_grp, c), wo_copy(c - c_wo - 1)])

    project_chunk(opaque_zero, 0, HG // 2, n_piece=0)
    request([w_copy(2, n_chunk - 1)])
    request_with_wo(range(c_wo + 1, c_wo + 3))
    w_wait(1)
    project_chunk(opaque_zero, 0, HG // 2, HG // 2)
    w_wait(2)

    @pl.loop(0, 2)
    def _(t):
        project_chunk(opaque_zero, 1, HG // 2, t * (HG // 2), n_rep // 2, t * (n_rep // 2))

    request_with_wo(range(c_wo + 3, n_ahead + 1))
    lax.fori_loop(1, c_wo // 2, functools.partial(pair_body, with_wo=False), 0)
    w_wait(n_chunk - 1)
    request([cp_x, cp_mem0, cp_wr, *cp_ffn])
    lax.fori_loop(c_wo // 2, n_ahead // 2, functools.partial(pair_body, with_wo=True), 0)
    for cp in (cp_x, cp_mem0, cp_wr):
        cp.wait()

    def project_tail(j, grp):
        half = GROUP * n_tail // 2
        rows = pl.ds(grp * half if isinstance(grp, int) else pl.multiple_of(grp * half, half), half)
        y = _dot(pltpu.bitcast(xt_v[rows, :], BF16), w_tile(j))
        stage[j // HG, pl.ds((j % HG) * n_seg + grp * GROUP, GROUP)] = (
            y.reshape(GROUP, n_tail, Dh).astype(BF16))

    late = range(n_ahead * HG, n_chunk * HG)
    for j in late:
        project_tail(j, 0)

    acc_v[...] = jnp.zeros(acc_v.shape, F32)
    acc_v[0:M, :] = mem0_v[...].astype(F32)
    r_at = (n_chunk, pl.ds(0, seg // HG))
    stage[r_at] = jnp.full((seg // HG, HG, LANES), -jnp.inf, BF16)

    def scores():
        return stage[r_at].astype(F32).reshape(seg, LANES)

    def norm_head(sg):
        xh_v[...] = _layernorm(x_v[sg].astype(F32)[:n_head])

    norm_head(0)

    def route(hn):
        w = wr_v[...].astype(F32)
        w = jnp.concatenate([w[i:i + 1] for i in range(w.shape[0])], axis=1)
        return _rb(jnp.sum(hn * w, axis=-1, keepdims=True))

    early = (n_seg - UNROLL - 1) * seg
    cp_early = pltpu.make_async_copy(out_v.at[pl.ds(0, early)], out_hbm.at[pl.ds(0, early)], sem_out[0])
    cp_late = pltpu.make_async_copy(out_v.at[pl.ds(early, S - early)],
                                    out_hbm.at[pl.ds(early, S - early)], sem_out[1])

    def finish_segment(sp, lane_id):
        rows = pl.ds(pl.multiple_of(sp * seg, seg), seg)
        h = _rb(x_v[sp].astype(F32) + _rb(acc_v[M:L, :]))
        hn = _layernorm(h)
        r = route(hn)
        h_v[rows, :] = h
        hn_v[rows, :] = hn
        out_v[rows, :] = (h + hn).astype(BF16)
        lane = lax.broadcasted_iota(jnp.int32, (seg, LANES), 1)
        r = jnp.where(lane == lane_id, r, scores())
        stage[r_at] = r.reshape(seg // HG, HG, LANES).astype(BF16)

    def step(s):
        lhs = jnp.concatenate([acc_v[0:M, :], xh_v[...]], axis=0).astype(BF16)
        norm_head(jnp.minimum(s + 1, n_seg - 1))
        qi = lax.broadcasted_iota(jnp.int32, (L, L), 0)
        ki = lax.broadcasted_iota(jnp.int32, (L, L), 1)
        visible = (qi < M) | (qi >= ki)

        def proj(m, h):
            j = m * H + h
            tail = stage[j // HG, (j % HG) * n_seg + s].astype(F32)
            return jnp.concatenate([_dot(lhs, w_tile(j)), tail], axis=0)

        val = {}
        acc = None
        for kind, h in _issue_order(H):
            if (kind, h) == ("q", 8):
                finish_segment(jnp.maximum(s - 1, 0), s - 1)
            if kind in "qkv":
                val[kind, h] = proj("qkv".index(kind), h)
            elif kind == "s":
                sc = _dot(val.pop(("q", h)), val.pop(("k", h)), NT) * (scale * LOG2E)
                sc = jnp.where(visible, sc, MASKED * LOG2E)
                ex = jnp.exp2(sc - jnp.max(sc, axis=-1, keepdims=True))
                val[kind, h] = ex, _recip(jnp.sum(ex, axis=-1, keepdims=True))
            elif kind == "p":
                ex, inv = val.pop(("s", h))
                val[kind, h] = _dot(ex, val.pop(("v", h))) * inv
            else:
                w = w_tile(3 * H + h)
                w = jnp.concatenate([w[t * Dh:(t + 1) * Dh] for t in range(n_col)], axis=1)
                y = _dot(val.pop(("p", h)), w)
                acc = y if acc is None else acc + y
        acc_v[...] = acc

    n_iter = n_seg // UNROLL

    def group(t, carry):
        pl.when(t == n_iter - 1)(cp_early.start)
        for u in range(UNROLL):
            step(t * UNROLL + u)
            gaps = min(GROUP, UNROLL - 1 - u // GROUP * GROUP)
            grp = jnp.minimum(t * (UNROLL // GROUP) + u // GROUP + 1, n_seg // GROUP - 1)
            for j in late[u % GROUP::gaps] if u < UNROLL - 1 else ():
                project_tail(j, grp)
        return carry

    lax.fori_loop(0, n_iter, group, 0)
    for cp in cp_ffn:
        cp.wait()
    finish_segment(n_seg - 1, n_seg - 1)
    cp_late.start()

    r = scores()
    pos = (lax.broadcasted_iota(jnp.int32, r.shape, 1) * seg
           + lax.broadcasted_iota(jnp.int32, r.shape, 0))
    last = seg * LANES - 1
    mag = (pltpu.bitcast(r, jnp.int32) >> 16) & 0x7FFF
    rank = jnp.where((r != r) | (pos >= S), 0, 0x8000 + jnp.where(r < 0, -mag, mag))
    key = pltpu.bitcast((1 << 30) + rank * (last + 1) + (last - pos), F32)
    key0 = jnp.max(key, keepdims=True)
    key1 = jnp.max(jnp.where(key == key0, 0.0, key), keepdims=True)
    i0, i1 = (jnp.clip(last - (lax.bitcast_convert_type(k, jnp.int32)[0, 0] & last), 0, S - 1)
              for k in (key0, key1))

    first = lax.broadcasted_iota(jnp.int32, (8, D), 0) == 0
    h_sel = jnp.where(first, h_v[pl.ds(i0, 1), :], h_v[pl.ds(i1, 1), :])
    hn_sel = jnp.where(first, hn_v[pl.ds(i0, 1), :], hn_v[pl.ds(i1, 1), :])
    r_sel = route(hn_sel)
    g = _rb(_dot(hn_sel, wg_v[...]))
    u = _rb(_dot(hn_sel, wu_v[...]))
    g = _rb(g * _rb(jax.nn.sigmoid(g)))
    y = _rb(_dot(_rb(g * u), wd_v[...]))
    y = _rb(y * _rb(jax.nn.sigmoid(r_sel)))
    new = h_sel + _rb(hn_sel + y)

    cp_early.wait()
    cp_late.wait()
    tile = 16
    fix = []
    for t, idx in enumerate((i0, i1)):
        start = pl.multiple_of((idx // tile) * tile, tile)
        rows = pl.ds(start, tile)
        hit = lax.broadcasted_iota(jnp.int32, (tile, D), 0) == idx - start
        out_v[rows, :] = jnp.where(hit, new[t:t + 1], out_v[rows, :].astype(F32)).astype(BF16)
        fix.append(pltpu.make_async_copy(out_v.at[rows], out_hbm.at[rows], sem_out[t]))
    two_tiles = i0 // tile != i1 // tile
    fix[0].start()
    pl.when(two_tiles)(fix[1].start)
    fix[0].wait()
    pl.when(two_tiles)(fix[1].wait)


@functools.partial(jax.jit, static_argnames=("A_seg_len",))
def pallas_sequential_preLN__memory_aug_recurrent_mem_tr__moe_arch_mod__prompt_kernel(
    A_x: jax.Array,
    A_mem0: jax.Array,
    A_Wq: jax.Array,
    A_Wk: jax.Array,
    A_Wv: jax.Array,
    A_Wo: jax.Array,
    A_seg_len: int,
    B_x: jax.Array,
    B_w_r: jax.Array,
    B_w_gate: jax.Array,
    B_w_up: jax.Array,
    B_w_down: jax.Array,
):
    del B_x
    B, S, D = A_x.shape
    M = A_mem0.shape[1]
    _, H, Dh = A_Wq.shape
    F = B_w_gate.shape[1]
    seg = int(A_seg_len)
    n_seg = S // seg
    assert B == 1 and Dh == LANES and n_seg <= LANES and S % (2 * seg) == 0 and H % HG == 0

    hbm = pl.BlockSpec(memory_space=pl.ANY)
    n_chunk = 3 * (H // HG)
    out = pl.pallas_call(
        _kernel,
        out_shape=jax.ShapeDtypeStruct((S, D), BF16),
        in_specs=[hbm] * 10,
        out_specs=hbm,
        scratch_shapes=[
            pltpu.VMEM((n_seg, seg, D), BF16),
            pltpu.VMEM((M, D), BF16),
            pltpu.VMEM((D // LANES, LANES), BF16),
            pltpu.VMEM((D, F), BF16),
            pltpu.VMEM((D, F), BF16),
            pltpu.VMEM((F, D), BF16),
            pltpu.VMEM((n_seg, M, D), BF16),
            pltpu.VMEM((seg - M, D), F32),
            pltpu.VMEM((n_seg * M // 2, D), U32),
            pltpu.VMEM((n_chunk + 1, D, HG, Dh), BF16),
            pltpu.VMEM((2 * H // HG, HG, D // 2, Dh), U32),
            pltpu.VMEM((2 * H // HG, HG, D // 2, Dh), U32),
            pltpu.VMEM((H, Dh, D), BF16),
            pltpu.VMEM((M + seg, D), F32),
            pltpu.VMEM((S, D), F32),
            pltpu.VMEM((S, D), F32),
            pltpu.VMEM((S, D), BF16),
            pltpu.SemaphoreType.DMA((n_chunk,)),
            pltpu.SemaphoreType.DMA((D // LANES,)),
            pltpu.SemaphoreType.DMA((H // HG,)),
            pltpu.SemaphoreType.DMA((9,)),
        ],
        compiler_params=pltpu.CompilerParams(vmem_limit_bytes=110 * 1024 * 1024),
        name="rmt_mod_block",
    )(
        A_x.reshape(n_seg, seg, D), A_mem0.reshape(M, D), A_Wq, A_Wk, A_Wv, A_Wo,
        B_w_r.reshape(D // LANES, LANES), B_w_gate, B_w_up, B_w_down,
    )
    return out.reshape(B, S, D)
```

```python
import functools

import jax
import jax.numpy as jnp
import numpy as np
from jax import lax
from jax.experimental import pallas as pl
from jax.experimental.pallas import tpu as pltpu

F32 = jnp.float32
BF16 = jnp.bfloat16
U32 = jnp.uint32
EPS = 1e-05
MASKED = -1000000000.0
LOG2E = 1.4426950408889634
NN = (((1,), (0,)), ((), ()))
NT = (((1,), (1,)), ((), ()))
LANES = 128
HG = 8
UNROLL = 8


def _rb(v):
    return v.astype(BF16).astype(F32)


def _layernorm(v):
    m = jnp.mean(v, axis=-1, keepdims=True)
    c = v - m
    var = jnp.mean(c * c, axis=-1, keepdims=True)
    sd = _rb(jnp.sqrt(_rb(_rb(var) + EPS)))
    return _rb(_rb(v - _rb(m)) / sd)


def _recip(v):
    r = pl.reciprocal(v, approx=True)
    return r + r * (1.0 - v * r)


def _dot(a, b, dims=NN):
    return lax.dot_general(a, b, dims, preferred_element_type=F32)


def _issue_order(n_heads):
    lag_v, lag_o = 7, 7
    cost = {"q": 32, "k": 32, "v": 32, "s": 10, "p": 10, "o": 40}
    lat_mxu, lat_softmax = 230, 480
    needs = {"s": (("k", lat_mxu),), "p": (("v", lat_mxu), ("s", lat_softmax)), "o": (("p", lat_mxu),)}
    proj = []
    for i in range(n_heads + lag_v):
        proj += [("q", i), ("k", i)] if i < n_heads else []
        proj += [("v", i - lag_v)] if i >= lag_v else []
    nxt = {"s": 0, "p": 0, "o": 0}
    done, order, now = {}, [], 0

    def ready_at(kind):
        h = nxt[kind]
        if h == n_heads or any((d, h) not in done for d, _ in needs[kind]):
            return None
        return max(done[d, h] + lat for d, lat in needs[kind])

    while len(order) < 6 * n_heads:
        at = {kind: ready_at(kind) for kind in nxt}
        if proj and ("v", min(nxt["o"] + lag_o, n_heads - 1)) not in done:
            at["o"] = None
        kinds = [kind for kind in nxt if at[kind] is not None]
        if not proj:
            now = max(now, min(at[kind] for kind in kinds))
        kinds = [kind for kind in kinds if at[kind] <= now]
        if kinds:
            op = (kinds[0], nxt[kinds[0]])
            nxt[kinds[0]] += 1
        else:
            op = proj.pop(0)
        now += cost[op[0]]
        done[op] = now
        order.append(op)
    return order


def _kernel(x_hbm, mem0_hbm, wq_hbm, wk_hbm, wv_hbm, wo_hbm, wr_hbm, wg_hbm, wu_hbm, wd_hbm,
            out_hbm,
            x_v, mem0_v, wr_v, wg_v, wu_v, wd_v, xt_raw, xh_v, xt_v, stage, w_even, w_odd, wo_raw,
            acc_v, h_v, hn_v, out_v, sem_w, sem_wo, sem):
    n_seg, seg, D = x_v.shape
    S = n_seg * seg
    M = mem0_v.shape[0]
    H, Dh, _ = wo_raw.shape
    L = M + seg
    n_tail = xt_raw.shape[1]
    n_head = seg - n_tail
    scale = Dh ** (-0.5)
    n_grp = H // HG
    n_chunk = 3 * n_grp
    n_ahead = n_chunk - 2
    c_wo = n_ahead - n_grp
    n_col = D // LANES
    n_rep = D // 16
    w_hbm = (wq_hbm, wk_hbm, wv_hbm)

    def w_copy(m, c):
        heads = pl.ds(pl.multiple_of((c - m * n_grp) * HG, HG), HG)
        return pltpu.make_async_copy(w_hbm[m].at[:, heads, :], stage.at[c], sem_w.at[c])

    def w_wait(c):
        if isinstance(c, int):
            w_copy(c // n_grp, c).wait()
        else:
            for m in range(3):
                pl.when(c // n_grp == m)(functools.partial(lambda m: w_copy(m, c).wait(), m))

    def first_copy(t):
        rows = pl.ds(t * LANES, LANES)
        return pltpu.make_async_copy(wq_hbm.at[rows, pl.ds(0, HG), :], stage.at[0, rows],
                                     sem_w.at[n_chunk + t])

    def wo_copy(g):
        heads = pl.ds(g * HG, HG)
        return pltpu.make_async_copy(wo_hbm.at[heads], wo_raw.at[heads], sem_wo.at[g])

    cp_tail = pltpu.make_async_copy(x_hbm.at[:, pl.ds(n_head, n_tail), :], xt_raw, sem_w.at[0])
    cp_x, cp_mem0, cp_wr, *cp_ffn = [
        pltpu.make_async_copy(src, dst, sem.at[i])
        for i, (src, dst) in enumerate(((x_hbm, x_v), (mem0_hbm, mem0_v), (wr_hbm, wr_v),
                                        (wg_hbm, wg_v), (wu_hbm, wu_v), (wd_hbm, wd_v)))
    ]
    sem_out = (sem.at[6], sem.at[7])

    def request(copies):
        for cp in copies:
            cp.start()

    cp_tail.start()
    request(first_copy(t) for t in range(n_col))
    request(w_copy(c // n_grp, c) for c in range(1, c_wo + 1))

    cp_tail.wait()
    xt = _layernorm(xt_raw[...].astype(F32).reshape(n_seg * n_tail, D))
    xt_v[...] = pltpu.bitcast(xt.astype(BF16), U32)

    w_buf = (w_even, w_odd)

    def repack(src, dst, slot, i):
        v = stage[src, pl.ds(i * 16, 16)]
        v = pltpu.bitcast(v.reshape(16 * HG, Dh), U32)
        v = jnp.swapaxes(v.reshape(8, HG, Dh), 0, 1)
        rows = pl.ds(i * 8, 8) if isinstance(i, int) else pl.ds(pl.multiple_of(i * 8, 8), 8)
        for j in range(HG // 2):
            a, b = v[j], v[HG // 2 + j]
            dst[slot, 2 * j, rows, :] = (a & 0xFFFF) | (b << 16)
            dst[slot, 2 * j + 1, rows, :] = (a >> 16) | (b & np.uint32(0xFFFF0000))

    def w_tile(j):
        c = j // HG
        return pltpu.bitcast(w_buf[c % 2][c // 2, j % HG], BF16)

    def first_body(t, carry):
        first_copy(t).wait()
        for i in range(n_rep // n_col):
            repack(0, w_even, 0, t * (n_rep // n_col) + i)
        return t

    pair0 = lax.fori_loop(0, n_col, first_body, 0) // n_col

    def project_chunk(p, par, n_heads=HG, head0=0, n_piece=n_rep, piece0=0, per_head=None):
        src = jnp.minimum(2 * p + par + 1, n_ahead)
        n_part = 16
        part = n_seg // n_part
        n_slot = n_heads * n_part - n_part // 2
        for k in range(n_heads):
            i = head0 + k
            y = _dot(pltpu.bitcast(xt_v[...], BF16), pltpu.bitcast(w_buf[par][p, i], BF16))
            y = y.reshape(n_seg, n_tail, Dh).astype(BF16)
            if per_head is not None:
                per_head(i)
            for t in range(n_part):
                at = k * n_part + t
                for r in range(n_piece)[at * n_piece // n_slot:(at + 1) * n_piece // n_slot]:
                    repack(src, w_buf[1 - par], p + par, piece0 + r)
                stage[2 * p + par, pl.ds(i * n_seg + t * part, part)] = y[t * part:(t + 1) * part]

    def pair_body(p, carry, *, with_wo):
        def extra(i):
            g = 2 * p - c_wo
            slot = jnp.minimum((n_chunk - c_wo) // 2 + p, 2 * n_grp - 1)
            for t in range(2):
                w = pltpu.bitcast(wo_raw[(g + t) * HG + i], U32)
                w_buf[t][slot, i] = jnp.concatenate(
                    [w[:, n * LANES:(n + 1) * LANES] for n in range(n_col)], axis=0)
                repack(n_chunk - 1, w_odd, n_chunk // 2 - 1, (g + t) * HG + i)

        for par in range(2):
            w_wait(2 * p + par + 1)
            if with_wo:
                wo_copy(2 * p + par - c_wo).wait()
        for par in range(2):
            project_chunk(p, par, per_head=extra if with_wo and par == 0 else None)
        return carry

    def request_with_wo(chunks):
        for c in chunks:
            request([w_copy(c // n_grp, c), wo_copy(c - c_wo - 1)])

    project_chunk(pair0, 0, HG // 2, n_piece=0)
    request([w_copy(2, n_chunk - 1)])
    request_with_wo(range(c_wo + 1, c_wo + 3))
    w_wait(1)
    project_chunk(pair0, 0, HG // 2, HG // 2)
    w_wait(2)

    @pl.loop(0, 2)
    def _(t):
        project_chunk(pair0, 1, HG // 2, t * (HG // 2), n_rep // 2, t * (n_rep // 2))

    request_with_wo(range(c_wo + 3, n_ahead + 1))
    lax.fori_loop(1, c_wo // 2, functools.partial(pair_body, with_wo=False), 0)
    w_wait(n_chunk - 1)
    request([cp_x, cp_mem0, cp_wr, *cp_ffn])
    lax.fori_loop(c_wo // 2, n_ahead // 2, functools.partial(pair_body, with_wo=True), 0)
    for cp in (cp_x, cp_mem0, cp_wr):
        cp.wait()

    def project_tail(j, grp):
        half = UNROLL * n_tail // 2
        rows = pl.ds(grp * half if isinstance(grp, int) else pl.multiple_of(grp * half, half), half)
        y = _dot(pltpu.bitcast(xt_v[rows, :], BF16), w_tile(j))
        stage[j // HG, pl.ds((j % HG) * n_seg + grp * UNROLL, UNROLL)] = (
            y.reshape(UNROLL, n_tail, Dh).astype(BF16))

    late = range(n_ahead * HG, n_chunk * HG)
    for j in late:
        project_tail(j, 0)

    acc_v[...] = jnp.zeros(acc_v.shape, F32)
    acc_v[0:M, :] = mem0_v[...].astype(F32)
    r_at = (n_chunk, pl.ds(0, seg // HG))
    stage[r_at] = jnp.full((seg // HG, HG, LANES), -jnp.inf, BF16)

    def scores():
        return stage[r_at].astype(F32).reshape(seg, LANES)

    def norm_head(sg):
        xh_v[...] = _layernorm(x_v[sg].astype(F32)[:n_head])

    norm_head(0)

    def route(hn):
        w = wr_v[...].astype(F32)
        w = jnp.concatenate([w[i:i + 1] for i in range(w.shape[0])], axis=1)
        return _rb(jnp.sum(hn * w, axis=-1, keepdims=True))

    early = (n_seg - UNROLL - 1) * seg
    cp_early = pltpu.make_async_copy(out_v.at[pl.ds(0, early)], out_hbm.at[pl.ds(0, early)], sem_out[0])
    cp_late = pltpu.make_async_copy(out_v.at[pl.ds(early, S - early)],
                                    out_hbm.at[pl.ds(early, S - early)], sem_out[1])

    def finish_segment(sp, lane_id):
        rows = pl.ds(pl.multiple_of(sp * seg, seg), seg)
        h = _rb(x_v[sp].astype(F32) + _rb(acc_v[M:L, :]))
        hn = _layernorm(h)
        r = route(hn)
        h_v[rows, :] = h
        hn_v[rows, :] = hn
        out_v[rows, :] = (h + hn).astype(BF16)
        lane = lax.broadcasted_iota(jnp.int32, (seg, LANES), 1)
        r = jnp.where(lane == lane_id, r, scores())
        stage[r_at] = r.reshape(seg // HG, HG, LANES).astype(BF16)

    def step(s):
        lhs = jnp.concatenate([acc_v[0:M, :], xh_v[...]], axis=0).astype(BF16)
        norm_head(jnp.minimum(s + 1, n_seg - 1))
        qi = lax.broadcasted_iota(jnp.int32, (L, L), 0)
        ki = lax.broadcasted_iota(jnp.int32, (L, L), 1)
        visible = (qi < M) | (qi >= ki)

        def proj(m, h):
            j = m * H + h
            tail = stage[j // HG, (j % HG) * n_seg + s].astype(F32)
            return jnp.concatenate([_dot(lhs, w_tile(j)), tail], axis=0)

        val = {}
        acc = None
        for kind, h in _issue_order(H):
            if (kind, h) == ("q", 8):
                finish_segment(jnp.maximum(s - 1, 0), s - 1)
            if kind in "qkv":
                val[kind, h] = proj("qkv".index(kind), h)
            elif kind == "s":
                sc = _dot(val.pop(("q", h)), val.pop(("k", h)), NT) * (scale * LOG2E)
                sc = jnp.where(visible, sc, MASKED * LOG2E)
                ex = jnp.exp2(sc - jnp.max(sc, axis=-1, keepdims=True))
                val[kind, h] = ex, _recip(jnp.sum(ex, axis=-1, keepdims=True))
            elif kind == "p":
                ex, inv = val.pop(("s", h))
                val[kind, h] = _dot(ex, val.pop(("v", h))) * inv
            else:
                w = w_tile(3 * H + h)
                w = jnp.concatenate([w[t * Dh:(t + 1) * Dh] for t in range(n_col)], axis=1)
                y = _dot(val.pop(("p", h)), w)
                acc = y if acc is None else acc + y
        acc_v[...] = acc

    n_iter = n_seg // UNROLL

    def group(t, carry):
        pl.when(t == n_iter - 1)(cp_early.start)
        for u in range(UNROLL):
            step(t * UNROLL + u)
            for j in late[u::UNROLL - 1] if u < UNROLL - 1 else ():
                project_tail(j, jnp.minimum(t + 1, n_iter - 1))
        return carry

    lax.fori_loop(0, n_iter, group, 0)
    for cp in cp_ffn:
        cp.wait()
    finish_segment(n_seg - 1, n_seg - 1)
    cp_late.start()

    r = scores()
    pos = (lax.broadcasted_iota(jnp.int32, r.shape, 1) * seg
           + lax.broadcasted_iota(jnp.int32, r.shape, 0))
    last = seg * LANES - 1
    mag = (pltpu.bitcast(r, jnp.int32) >> 16) & 0x7FFF
    rank = jnp.where((r != r) | (pos >= S), 0, 0x8000 + jnp.where(r < 0, -mag, mag))
    key = pltpu.bitcast((1 << 30) + rank * (last + 1) + (last - pos), F32)
    key0 = jnp.max(key, keepdims=True)
    key1 = jnp.max(jnp.where(key == key0, 0.0, key), keepdims=True)
    i0, i1 = (jnp.clip(last - (lax.bitcast_convert_type(k, jnp.int32)[0, 0] & last), 0, S - 1)
              for k in (key0, key1))

    first = lax.broadcasted_iota(jnp.int32, (8, D), 0) == 0
    h_sel = jnp.where(first, h_v[pl.ds(i0, 1), :], h_v[pl.ds(i1, 1), :])
    hn_sel = jnp.where(first, hn_v[pl.ds(i0, 1), :], hn_v[pl.ds(i1, 1), :])
    r_sel = route(hn_sel)
    g = _rb(_dot(hn_sel, wg_v[...]))
    u = _rb(_dot(hn_sel, wu_v[...]))
    g = _rb(g * _rb(jax.nn.sigmoid(g)))
    y = _rb(_dot(_rb(g * u), wd_v[...]))
    y = _rb(y * _rb(jax.nn.sigmoid(r_sel)))
    new = h_sel + _rb(hn_sel + y)

    cp_early.wait()
    cp_late.wait()
    tile = 16
    fix = []
    for t, idx in enumerate((i0, i1)):
        start = pl.multiple_of((idx // tile) * tile, tile)
        rows = pl.ds(start, tile)
        hit = lax.broadcasted_iota(jnp.int32, (tile, D), 0) == idx - start
        out_v[rows, :] = jnp.where(hit, new[t:t + 1], out_v[rows, :].astype(F32)).astype(BF16)
        fix.append(pltpu.make_async_copy(out_v.at[rows], out_hbm.at[rows], sem_out[t]))
    two_tiles = i0 // tile != i1 // tile
    fix[0].start()
    pl.when(two_tiles)(fix[1].start)
    fix[0].wait()
    pl.when(two_tiles)(fix[1].wait)


@functools.partial(jax.jit, static_argnames=("A_seg_len",))
def pallas_sequential_preLN__memory_aug_recurrent_mem_tr__moe_arch_mod__prompt_kernel(
    A_x: jax.Array,
    A_mem0: jax.Array,
    A_Wq: jax.Array,
    A_Wk: jax.Array,
    A_Wv: jax.Array,
    A_Wo: jax.Array,
    A_seg_len: int,
    B_x: jax.Array,
    B_w_r: jax.Array,
    B_w_gate: jax.Array,
    B_w_up: jax.Array,
    B_w_down: jax.Array,
):
    del B_x
    B, S, D = A_x.shape
    M = A_mem0.shape[1]
    _, H, Dh = A_Wq.shape
    F = B_w_gate.shape[1]
    seg = int(A_seg_len)
    n_seg = S // seg
    assert (B, S, D, M, H, Dh, seg) == (1, 2048, 512, 8, 32, LANES, 32)

    hbm = pl.BlockSpec(memory_space=pl.ANY)
    n_chunk = 3 * (H // HG)
    out = pl.pallas_call(
        _kernel,
        out_shape=jax.ShapeDtypeStruct((S, D), BF16),
        in_specs=[hbm] * 10,
        out_specs=hbm,
        scratch_shapes=[
            pltpu.VMEM((n_seg, seg, D), BF16),
            pltpu.VMEM((M, D), BF16),
            pltpu.VMEM((D // LANES, LANES), BF16),
            pltpu.VMEM((D, F), BF16),
            pltpu.VMEM((D, F), BF16),
            pltpu.VMEM((F, D), BF16),
            pltpu.VMEM((n_seg, M, D), BF16),
            pltpu.VMEM((seg - M, D), F32),
            pltpu.VMEM((n_seg * M // 2, D), U32),
            pltpu.VMEM((n_chunk + 1, D, HG, Dh), BF16),
            pltpu.VMEM((2 * H // HG, HG, D // 2, Dh), U32),
            pltpu.VMEM((2 * H // HG, HG, D // 2, Dh), U32),
            pltpu.VMEM((H, Dh, D), BF16),
            pltpu.VMEM((M + seg, D), F32),
            pltpu.VMEM((S, D), F32),
            pltpu.VMEM((S, D), F32),
            pltpu.VMEM((S, D), BF16),
            pltpu.SemaphoreType.DMA((n_chunk + D // LANES,)),
            pltpu.SemaphoreType.DMA((H // HG,)),
            pltpu.SemaphoreType.DMA((8,)),
        ],
        compiler_params=pltpu.CompilerParams(vmem_limit_bytes=110 * 1024 * 1024),
        name="rmt_mod_block",
    )(
        A_x.reshape(n_seg, seg, D), A_mem0.reshape(M, D), A_Wq, A_Wk, A_Wv, A_Wo,
        B_w_r.reshape(D // LANES, LANES), B_w_gate, B_w_up, B_w_down,
    )
    return out.reshape(B, S, D)
```

```python
import functools

import jax
import jax.numpy as jnp
import numpy as np
from jax import lax
from jax.experimental import pallas as pl
from jax.experimental.pallas import tpu as pltpu

F32 = jnp.float32
BF16 = jnp.bfloat16
U32 = jnp.uint32
EPS = 1e-05
MASKED = -1000000000.0
LOG2E = 1.4426950408889634
NN = (((1,), (0,)), ((), ()))
NT = (((1,), (1,)), ((), ()))
LANES = 128
HG = 8
UNROLL = 8


def _rb(v):
    return v.astype(BF16).astype(F32)


def _layernorm(v):
    m = jnp.mean(v, axis=-1, keepdims=True)
    c = v - m
    var = jnp.mean(c * c, axis=-1, keepdims=True)
    sd = _rb(jnp.sqrt(_rb(_rb(var) + EPS)))
    return _rb(_rb(v - _rb(m)) / sd)


def _recip(v):
    r = pl.reciprocal(v, approx=True)
    return r + r * (1.0 - v * r)


def _dot(a, b, dims=NN):
    return lax.dot_general(a, b, dims, preferred_element_type=F32)


def _issue_order(n_heads):
    lag_v, lag_o = 7, 7
    cost = {"q": 32, "k": 32, "v": 32, "s": 10, "p": 10, "o": 40}
    lat_mxu, lat_softmax = 230, 480
    needs = {"s": (("k", lat_mxu),), "p": (("v", lat_mxu), ("s", lat_softmax)), "o": (("p", lat_mxu),)}
    proj = []
    for i in range(n_heads + lag_v):
        proj += [("q", i), ("k", i)] if i < n_heads else []
        proj += [("v", i - lag_v)] if i >= lag_v else []
    nxt = {"s": 0, "p": 0, "o": 0}
    done, order, now = {}, [], 0

    def ready_at(kind):
        h = nxt[kind]
        if h == n_heads or any((d, h) not in done for d, _ in needs[kind]):
            return None
        return max(done[d, h] + lat for d, lat in needs[kind])

    while len(order) < 6 * n_heads:
        at = {kind: ready_at(kind) for kind in nxt}
        if proj and ("v", min(nxt["o"] + lag_o, n_heads - 1)) not in done:
            at["o"] = None
        kinds = [kind for kind in nxt if at[kind] is not None]
        if not proj:
            now = max(now, min(at[kind] for kind in kinds))
        kinds = [kind for kind in kinds if at[kind] <= now]
        if kinds:
            op = (kinds[0], nxt[kinds[0]])
            nxt[kinds[0]] += 1
        else:
            op = proj.pop(0)
        now += cost[op[0]]
        done[op] = now
        order.append(op)
    return order


def _kernel(x_hbm, mem0_hbm, wq_hbm, wk_hbm, wv_hbm, wo_hbm, wr_hbm, wg_hbm, wu_hbm, wd_hbm,
            out_hbm,
            x_v, mem0_v, wr_v, wg_v, wu_v, wd_v, xt_raw, xh_v, xt_v, stage, w_even, w_odd, wo_raw,
            acc_v, h_v, hn_v, out_v, sem_w, sem):
    n_seg, seg, D = x_v.shape
    S = n_seg * seg
    M = mem0_v.shape[0]
    H, Dh, _ = wo_raw.shape
    L = M + seg
    n_tail = xt_raw.shape[1]
    n_head = seg - n_tail
    scale = Dh ** (-0.5)
    n_grp = H // HG
    n_chunk = 3 * n_grp
    n_ahead = n_chunk - 2
    n_col = D // LANES
    n_rep = D // 16
    w_hbm = (wq_hbm, wk_hbm, wv_hbm)

    def w_copy(m, c):
        heads = pl.ds(pl.multiple_of((c - m * n_grp) * HG, HG), HG)
        return pltpu.make_async_copy(w_hbm[m].at[:, heads, :], stage.at[c], sem_w.at[c])

    def w_wait(c):
        if isinstance(c, int):
            w_copy(c // n_grp, c).wait()
        else:
            for m in range(3):
                pl.when(c // n_grp == m)(functools.partial(lambda m: w_copy(m, c).wait(), m))

    def part_copy(c, t):
        rows = pl.ds(t * LANES, LANES)
        src = w_hbm[c // n_grp].at[rows, pl.ds(c % n_grp * HG, HG), :]
        return pltpu.make_async_copy(src, stage.at[c, rows],
                                     sem_w.at[n_chunk + (n_col if c else 0) + t])

    cp_tail = pltpu.make_async_copy(x_hbm.at[:, pl.ds(n_head, n_tail), :], xt_raw, sem_w.at[0])
    *cp_rest, cp_gate, cp_up, cp_down = [
        pltpu.make_async_copy(src, dst, sem.at[i])
        for i, (src, dst) in enumerate((
            (wo_hbm, wo_raw), (x_hbm, x_v), (mem0_hbm, mem0_v), (wr_hbm, wr_v),
            (wg_hbm, wg_v), (wu_hbm, wu_v), (wd_hbm, wd_v)))
    ]
    cp_ffn = (cp_gate, cp_up, cp_down)
    sem_out = (sem.at[7], sem.at[8])

    def request(copies):
        for cp in copies:
            cp.start()

    cp_tail.start()
    request(part_copy(0, t) for t in range(n_col))
    for c in range(1, n_ahead + 1):
        w_copy(c // n_grp, c).start()
        if c % 2 == 0 and c > 2:
            part_copy(n_chunk - 1, c // 2 - 2).start()

    cp_tail.wait()
    xt = _layernorm(xt_raw[...].astype(F32).reshape(n_seg * n_tail, D))
    xt_v[...] = pltpu.bitcast(xt.astype(BF16), U32)

    w_buf = (w_even, w_odd)

    def repack(src, dst, slot, i):
        v = stage[src, pl.ds(i * 16, 16)]
        v = pltpu.bitcast(v.reshape(16 * HG, Dh), U32)
        v = jnp.swapaxes(v.reshape(8, HG, Dh), 0, 1)
        rows = pl.ds(i * 8, 8) if isinstance(i, int) else pl.ds(pl.multiple_of(i * 8, 8), 8)
        for j in range(HG // 2):
            a, b = v[j], v[HG // 2 + j]
            dst[slot, 2 * j, rows, :] = (a & 0xFFFF) | (b << 16)
            dst[slot, 2 * j + 1, rows, :] = (a >> 16) | (b & np.uint32(0xFFFF0000))

    def w_tile(j):
        c = j // HG
        return pltpu.bitcast(w_buf[c % 2][c // 2, j % HG], BF16)

    def first_body(t, carry):
        part_copy(0, t).wait()
        for i in range(n_rep // n_col):
            repack(0, w_even, 0, t * (n_rep // n_col) + i)
        return t

    pair0 = lax.fori_loop(0, n_col, first_body, 0) // n_col

    def project_chunk(p, par, n_heads=HG, head0=0, n_piece=n_rep, piece0=0, per_head=None):
        src = jnp.minimum(2 * p + par + 1, n_ahead)
        n_part = 16
        part = n_seg // n_part
        n_slot = n_heads * n_part - n_part // 2
        for k in range(n_heads):
            i = head0 + k
            y = _dot(pltpu.bitcast(xt_v[...], BF16), pltpu.bitcast(w_buf[par][p, i], BF16))
            y = y.reshape(n_seg, n_tail, Dh).astype(BF16)
            if per_head is not None:
                per_head(i)
            for t in range(n_part):
                at = k * n_part + t
                for r in range(n_piece)[at * n_piece // n_slot:(at + 1) * n_piece // n_slot]:
                    repack(src, w_buf[1 - par], p + par, piece0 + r)
                stage[2 * p + par, pl.ds(i * n_seg + t * part, part)] = y[t * part:(t + 1) * part]

    def pair_body(p, carry):
        for par in range(2):
            w_wait(2 * p + par + 1)
        part_copy(n_chunk - 1, p - 1).wait()
        project_chunk(p, 0, per_head=lambda i: repack(
            n_chunk - 1, w_odd, n_chunk // 2 - 1, (p - 1) * HG + i))
        project_chunk(p, 1)
        return carry

    project_chunk(pair0, 0, HG // 2, n_piece=0)
    w_wait(1)
    project_chunk(pair0, 0, HG // 2, HG // 2)
    w_wait(2)

    @pl.loop(0, 2)
    def _(t):
        project_chunk(pair0, 1, HG // 2, t * (HG // 2), n_rep // 2, t * (n_rep // 2))

    request((*cp_rest, *cp_ffn))
    lax.fori_loop(1, n_ahead // 2, pair_body, 0)
    for cp in cp_rest:
        cp.wait()

    def project_tail(j, grp):
        half = UNROLL * n_tail // 2
        rows = pl.ds(grp * half if isinstance(grp, int) else pl.multiple_of(grp * half, half), half)
        y = _dot(pltpu.bitcast(xt_v[rows, :], BF16), w_tile(j))
        stage[j // HG, pl.ds((j % HG) * n_seg + grp * UNROLL, UNROLL)] = (
            y.reshape(UNROLL, n_tail, Dh).astype(BF16))

    late = range(n_ahead * HG, n_chunk * HG)
    for j in late:
        project_tail(j, 0)
        for g in range(j // HG % 2, n_grp, 2):
            w = pltpu.bitcast(wo_raw[g * HG + j % HG], U32)
            w_buf[g % 2][pair0 + (n_chunk + g) // 2, j % HG] = jnp.concatenate(
                [w[:, n * LANES:(n + 1) * LANES] for n in range(n_col)], axis=0)

    acc_v[...] = jnp.zeros(acc_v.shape, F32)
    acc_v[0:M, :] = mem0_v[...].astype(F32)
    r_at = (n_chunk, pl.ds(0, seg // HG))
    stage[r_at] = jnp.full((seg // HG, HG, LANES), -jnp.inf, BF16)

    def scores():
        return stage[r_at].astype(F32).reshape(seg, LANES)

    def norm_head(sg):
        xh_v[...] = _layernorm(x_v[sg].astype(F32)[:n_head])

    norm_head(0)

    def route(hn):
        w = wr_v[...].astype(F32)
        w = jnp.concatenate([w[i:i + 1] for i in range(w.shape[0])], axis=1)
        return _rb(jnp.sum(hn * w, axis=-1, keepdims=True))

    early = (n_seg - UNROLL - 1) * seg
    cp_early = pltpu.make_async_copy(out_v.at[pl.ds(0, early)], out_hbm.at[pl.ds(0, early)], sem_out[0])
    cp_late = pltpu.make_async_copy(out_v.at[pl.ds(early, S - early)],
                                    out_hbm.at[pl.ds(early, S - early)], sem_out[1])

    def finish_segment(sp, lane_id):
        rows = pl.ds(pl.multiple_of(sp * seg, seg), seg)
        h = _rb(x_v[sp].astype(F32) + _rb(acc_v[M:L, :]))
        hn = _layernorm(h)
        r = route(hn)
        h_v[rows, :] = h
        hn_v[rows, :] = hn
        out_v[rows, :] = (h + hn).astype(BF16)
        lane = lax.broadcasted_iota(jnp.int32, (seg, LANES), 1)
        r = jnp.where(lane == lane_id, r, scores())
        stage[r_at] = r.reshape(seg // HG, HG, LANES).astype(BF16)

    def step(s):
        lhs = jnp.concatenate([acc_v[0:M, :], xh_v[...]], axis=0).astype(BF16)
        norm_head(jnp.minimum(s + 1, n_seg - 1))
        qi = lax.broadcasted_iota(jnp.int32, (L, L), 0)
        ki = lax.broadcasted_iota(jnp.int32, (L, L), 1)
        visible = (qi < M) | (qi >= ki)

        def proj(m, h):
            j = m * H + h
            tail = stage[j // HG, (j % HG) * n_seg + s].astype(F32)
            return jnp.concatenate([_dot(lhs, w_tile(j)), tail], axis=0)

        val = {}
        acc = None
        for kind, h in _issue_order(H):
            if (kind, h) == ("q", 8):
                finish_segment(jnp.maximum(s - 1, 0), s - 1)
            if kind in "qkv":
                val[kind, h] = proj("qkv".index(kind), h)
            elif kind == "s":
                sc = _dot(val.pop(("q", h)), val.pop(("k", h)), NT) * (scale * LOG2E)
                sc = jnp.where(visible, sc, MASKED * LOG2E)
                ex = jnp.exp2(sc - jnp.max(sc, axis=-1, keepdims=True))
                val[kind, h] = ex, _recip(jnp.sum(ex, axis=-1, keepdims=True))
            elif kind == "p":
                ex, inv = val.pop(("s", h))
                val[kind, h] = _dot(ex, val.pop(("v", h))) * inv
            else:
                w = w_tile(3 * H + h)
                w = jnp.concatenate([w[t * Dh:(t + 1) * Dh] for t in range(n_col)], axis=1)
                y = _dot(val.pop(("p", h)), w)
                acc = y if acc is None else acc + y
        acc_v[...] = acc

    n_iter = n_seg // UNROLL

    def group(t, carry):
        pl.when(t == n_iter - 1)(cp_early.start)
        for u in range(UNROLL):
            step(t * UNROLL + u)
            for j in late[u::UNROLL - 1] if u < UNROLL - 1 else ():
                project_tail(j, jnp.minimum(t + 1, n_iter - 1))
        return carry

    lax.fori_loop(0, n_iter, group, 0)
    for cp in cp_ffn:
        cp.wait()
    finish_segment(n_seg - 1, n_seg - 1)
    cp_late.start()

    r = scores()
    pos = (lax.broadcasted_iota(jnp.int32, r.shape, 1) * seg
           + lax.broadcasted_iota(jnp.int32, r.shape, 0))
    last = seg * LANES - 1
    mag = (pltpu.bitcast(r, jnp.int32) >> 16) & 0x7FFF
    rank = jnp.where((r != r) | (pos >= S), 0, 0x8000 + jnp.where(r < 0, -mag, mag))
    key = pltpu.bitcast((1 << 30) + rank * (last + 1) + (last - pos), F32)
    key0 = jnp.max(key, keepdims=True)
    key1 = jnp.max(jnp.where(key == key0, 0.0, key), keepdims=True)
    i0, i1 = (jnp.clip(last - (lax.bitcast_convert_type(k, jnp.int32)[0, 0] & last), 0, S - 1)
              for k in (key0, key1))

    first = lax.broadcasted_iota(jnp.int32, (8, D), 0) == 0
    h_sel = jnp.where(first, h_v[pl.ds(i0, 1), :], h_v[pl.ds(i1, 1), :])
    hn_sel = jnp.where(first, hn_v[pl.ds(i0, 1), :], hn_v[pl.ds(i1, 1), :])
    r_sel = route(hn_sel)
    g = _rb(_dot(hn_sel, wg_v[...]))
    u = _rb(_dot(hn_sel, wu_v[...]))
    g = _rb(g * _rb(jax.nn.sigmoid(g)))
    y = _rb(_dot(_rb(g * u), wd_v[...]))
    y = _rb(y * _rb(jax.nn.sigmoid(r_sel)))
    new = h_sel + _rb(hn_sel + y)

    cp_early.wait()
    cp_late.wait()
    tile = 16
    fix = []
    for t, idx in enumerate((i0, i1)):
        start = pl.multiple_of((idx // tile) * tile, tile)
        rows = pl.ds(start, tile)
        hit = lax.broadcasted_iota(jnp.int32, (tile, D), 0) == idx - start
        out_v[rows, :] = jnp.where(hit, new[t:t + 1], out_v[rows, :].astype(F32)).astype(BF16)
        fix.append(pltpu.make_async_copy(out_v.at[rows], out_hbm.at[rows], sem_out[t]))
    two_tiles = i0 // tile != i1 // tile
    fix[0].start()
    pl.when(two_tiles)(fix[1].start)
    fix[0].wait()
    pl.when(two_tiles)(fix[1].wait)


@functools.partial(jax.jit, static_argnames=("A_seg_len",))
def pallas_sequential_preLN__memory_aug_recurrent_mem_tr__moe_arch_mod__prompt_kernel(
    A_x: jax.Array,
    A_mem0: jax.Array,
    A_Wq: jax.Array,
    A_Wk: jax.Array,
    A_Wv: jax.Array,
    A_Wo: jax.Array,
    A_seg_len: int,
    B_x: jax.Array,
    B_w_r: jax.Array,
    B_w_gate: jax.Array,
    B_w_up: jax.Array,
    B_w_down: jax.Array,
):
    del B_x
    B, S, D = A_x.shape
    M = A_mem0.shape[1]
    _, H, Dh = A_Wq.shape
    F = B_w_gate.shape[1]
    seg = int(A_seg_len)
    n_seg = S // seg
    assert (B, S, D, M, H, Dh, seg) == (1, 2048, 512, 8, 32, LANES, 32)

    hbm = pl.BlockSpec(memory_space=pl.ANY)
    n_chunk = 3 * (H // HG)
    out = pl.pallas_call(
        _kernel,
        out_shape=jax.ShapeDtypeStruct((S, D), BF16),
        in_specs=[hbm] * 10,
        out_specs=hbm,
        scratch_shapes=[
            pltpu.VMEM((n_seg, seg, D), BF16),
            pltpu.VMEM((M, D), BF16),
            pltpu.VMEM((D // LANES, LANES), BF16),
            pltpu.VMEM((D, F), BF16),
            pltpu.VMEM((D, F), BF16),
            pltpu.VMEM((F, D), BF16),
            pltpu.VMEM((n_seg, M, D), BF16),
            pltpu.VMEM((seg - M, D), F32),
            pltpu.VMEM((n_seg * M // 2, D), U32),
            pltpu.VMEM((n_chunk + 1, D, HG, Dh), BF16),
            pltpu.VMEM((2 * H // HG, HG, D // 2, Dh), U32),
            pltpu.VMEM((2 * H // HG, HG, D // 2, Dh), U32),
            pltpu.VMEM((H, Dh, D), BF16),
            pltpu.VMEM((M + seg, D), F32),
            pltpu.VMEM((S, D), F32),
            pltpu.VMEM((S, D), F32),
            pltpu.VMEM((S, D), BF16),
            pltpu.SemaphoreType.DMA((n_chunk + 2 * D // LANES,)),
            pltpu.SemaphoreType.DMA((9,)),
        ],
        compiler_params=pltpu.CompilerParams(vmem_limit_bytes=110 * 1024 * 1024),
        name="rmt_mod_block",
    )(
        A_x.reshape(n_seg, seg, D), A_mem0.reshape(M, D), A_Wq, A_Wk, A_Wv, A_Wo,
        B_w_r.reshape(D // LANES, LANES), B_w_gate, B_w_up, B_w_down,
    )
    return out.reshape(B, S, D)
```

```python
import functools

import jax
import jax.numpy as jnp
import numpy as np
from jax import lax
from jax.experimental import pallas as pl
from jax.experimental.pallas import tpu as pltpu

F32 = jnp.float32
BF16 = jnp.bfloat16
U32 = jnp.uint32
EPS = 1e-05
MASKED = -1000000000.0
LOG2E = 1.4426950408889634
NN = (((1,), (0,)), ((), ()))
NT = (((1,), (1,)), ((), ()))
LANES = 128
HG = 8
UNROLL = 8


def _rb(v):
    return v.astype(BF16).astype(F32)


def _layernorm(v):
    m = jnp.mean(v, axis=-1, keepdims=True)
    c = v - m
    var = jnp.mean(c * c, axis=-1, keepdims=True)
    sd = _rb(jnp.sqrt(_rb(_rb(var) + EPS)))
    return _rb(_rb(v - _rb(m)) / sd)


def _recip(v):
    r = pl.reciprocal(v, approx=True)
    return r + r * (1.0 - v * r)


def _dot(a, b, dims=NN):
    return lax.dot_general(a, b, dims, preferred_element_type=F32)


def _issue_order(n_heads):
    lag_v, lag_o = 7, 7
    cost = {"q": 32, "k": 32, "v": 32, "s": 10, "p": 10, "o": 40}
    lat_mxu, lat_softmax = 230, 480
    needs = {"s": (("k", lat_mxu),), "p": (("v", lat_mxu), ("s", lat_softmax)), "o": (("p", lat_mxu),)}
    proj = []
    for i in range(n_heads + lag_v):
        proj += [("q", i), ("k", i)] if i < n_heads else []
        proj += [("v", i - lag_v)] if i >= lag_v else []
    nxt = {"s": 0, "p": 0, "o": 0}
    done, order, now = {}, [], 0

    def ready_at(kind):
        h = nxt[kind]
        if h == n_heads or any((d, h) not in done for d, _ in needs[kind]):
            return None
        return max(done[d, h] + lat for d, lat in needs[kind])

    while len(order) < 6 * n_heads:
        at = {kind: ready_at(kind) for kind in nxt}
        if proj and ("v", min(nxt["o"] + lag_o, n_heads - 1)) not in done:
            at["o"] = None
        kinds = [kind for kind in nxt if at[kind] is not None]
        if not proj:
            now = max(now, min(at[kind] for kind in kinds))
        kinds = [kind for kind in kinds if at[kind] <= now]
        if kinds:
            op = (kinds[0], nxt[kinds[0]])
            nxt[kinds[0]] += 1
        else:
            op = proj.pop(0)
        now += cost[op[0]]
        done[op] = now
        order.append(op)
    return order


def _kernel(x_hbm, mem0_hbm, wq_hbm, wk_hbm, wv_hbm, wo_hbm, wr_hbm, wg_hbm, wu_hbm, wd_hbm,
            out_hbm,
            x_v, mem0_v, wr_v, wg_v, wu_v, wd_v, xt_raw, xh_v, xt_v, stage, w_even, w_odd, wo_raw,
            acc_v, h_v, hn_v, out_v, sem_w, sem):
    n_seg, seg, D = x_v.shape
    S = n_seg * seg
    M = mem0_v.shape[0]
    H, Dh, _ = wo_raw.shape
    L = M + seg
    n_tail = xt_raw.shape[1]
    n_head = seg - n_tail
    scale = Dh ** (-0.5)
    n_grp = H // HG
    n_chunk = 3 * n_grp
    n_ahead = n_chunk - 2
    n_col = D // LANES
    n_rep = D // 16
    w_hbm = (wq_hbm, wk_hbm, wv_hbm)

    def w_copy(m, c):
        heads = pl.ds(pl.multiple_of((c - m * n_grp) * HG, HG), HG)
        return pltpu.make_async_copy(w_hbm[m].at[:, heads, :], stage.at[c], sem_w.at[c])

    def w_wait(c):
        if isinstance(c, int):
            w_copy(c // n_grp, c).wait()
        else:
            for m in range(3):
                pl.when(c // n_grp == m)(functools.partial(lambda m: w_copy(m, c).wait(), m))

    def part_copy(c, t):
        rows = pl.ds(t * LANES, LANES)
        src = w_hbm[c // n_grp].at[rows, pl.ds(c % n_grp * HG, HG), :]
        return pltpu.make_async_copy(src, stage.at[c, rows],
                                     sem_w.at[n_chunk + (n_col if c else 0) + t])

    cp_tail = pltpu.make_async_copy(x_hbm.at[:, pl.ds(n_head, n_tail), :], xt_raw, sem_w.at[0])
    *cp_rest, cp_gate, cp_up, cp_down = [
        pltpu.make_async_copy(src, dst, sem.at[i])
        for i, (src, dst) in enumerate((
            (wo_hbm, wo_raw), (x_hbm, x_v), (mem0_hbm, mem0_v), (wr_hbm, wr_v),
            (wg_hbm, wg_v), (wu_hbm, wu_v), (wd_hbm, wd_v)))
    ]
    cp_ffn = (cp_gate, cp_up, cp_down)
    sem_out = (sem.at[7], sem.at[8])

    def request(copies):
        for cp in copies:
            cp.start()

    cp_tail.start()
    request(part_copy(0, t) for t in range(n_col))
    for c in range(1, n_ahead + 1):
        w_copy(c // n_grp, c).start()
        if c % 2 == 0 and c > 2:
            part_copy(n_chunk - 1, c // 2 - 2).start()

    cp_tail.wait()
    xt = _layernorm(xt_raw[...].astype(F32).reshape(n_seg * n_tail, D))
    xt_v[...] = pltpu.bitcast(xt.astype(BF16), U32)

    w_buf = (w_even, w_odd)

    def repack(src, dst, slot, i):
        v = stage[src, pl.ds(i * 16, 16)]
        v = pltpu.bitcast(v.reshape(16 * HG, Dh), U32)
        v = jnp.swapaxes(v.reshape(8, HG, Dh), 0, 1)
        rows = pl.ds(i * 8, 8) if isinstance(i, int) else pl.ds(pl.multiple_of(i * 8, 8), 8)
        for j in range(HG // 2):
            a, b = v[j], v[HG // 2 + j]
            dst[slot, 2 * j, rows, :] = (a & 0xFFFF) | (b << 16)
            dst[slot, 2 * j + 1, rows, :] = (a >> 16) | (b & np.uint32(0xFFFF0000))

    def w_tile(j):
        c = j // HG
        return pltpu.bitcast(w_buf[c % 2][c // 2, j % HG], BF16)

    def first_body(t, carry):
        part_copy(0, t).wait()
        for i in range(n_rep // n_col):
            repack(0, w_even, 0, t * (n_rep // n_col) + i)
        return t

    pair0 = lax.fori_loop(0, n_col, first_body, 0) // n_col

    def project_chunk(p, par, n_heads=HG, head0=0, n_piece=n_rep, per_head=None):
        src = jnp.minimum(2 * p + par + 1, n_ahead)
        n_part = 16
        part = n_seg // n_part
        n_slot = n_heads * n_part - n_part // 2
        for k in range(n_heads):
            i = head0 + k
            y = _dot(pltpu.bitcast(xt_v[...], BF16), pltpu.bitcast(w_buf[par][p, i], BF16))
            y = y.reshape(n_seg, n_tail, Dh).astype(BF16)
            if per_head is not None:
                per_head(i)
            for t in range(n_part):
                at = k * n_part + t
                for r in range(n_piece)[at * n_piece // n_slot:(at + 1) * n_piece // n_slot]:
                    repack(src, w_buf[1 - par], p + par, r)
                stage[2 * p + par, pl.ds(i * n_seg + t * part, part)] = y[t * part:(t + 1) * part]

    def pair_body(p, carry):
        for par in range(2):
            w_wait(2 * p + par + 1)
        part_copy(n_chunk - 1, p - 1).wait()
        project_chunk(p, 0, per_head=lambda i: repack(
            n_chunk - 1, w_odd, n_chunk // 2 - 1, (p - 1) * HG + i))
        project_chunk(p, 1)
        return carry

    project_chunk(pair0, 0, HG // 2, n_piece=0)
    w_wait(1)
    project_chunk(pair0, 0, HG // 2, HG // 2)
    w_wait(2)
    project_chunk(pair0, 1)
    request((*cp_rest, *cp_ffn))
    lax.fori_loop(1, n_ahead // 2, pair_body, 0)
    for cp in cp_rest:
        cp.wait()

    def project_tail(j, grp):
        half = UNROLL * n_tail // 2
        rows = pl.ds(grp * half if isinstance(grp, int) else pl.multiple_of(grp * half, half), half)
        y = _dot(pltpu.bitcast(xt_v[rows, :], BF16), w_tile(j))
        stage[j // HG, pl.ds((j % HG) * n_seg + grp * UNROLL, UNROLL)] = (
            y.reshape(UNROLL, n_tail, Dh).astype(BF16))

    late = range(n_ahead * HG, n_chunk * HG)
    for j in late:
        project_tail(j, 0)
        for g in range(j // HG % 2, n_grp, 2):
            w = pltpu.bitcast(wo_raw[g * HG + j % HG], U32)
            w_buf[g % 2][pair0 + (n_chunk + g) // 2, j % HG] = jnp.concatenate(
                [w[:, n * LANES:(n + 1) * LANES] for n in range(n_col)], axis=0)

    acc_v[...] = jnp.zeros(acc_v.shape, F32)
    acc_v[0:M, :] = mem0_v[...].astype(F32)
    r_at = (n_chunk, pl.ds(0, seg // HG))
    stage[r_at] = jnp.full((seg // HG, HG, LANES), -jnp.inf, BF16)

    def scores():
        return stage[r_at].astype(F32).reshape(seg, LANES)

    def norm_head(sg):
        xh_v[...] = _layernorm(x_v[sg].astype(F32)[:n_head])

    norm_head(0)

    def route(hn):
        w = wr_v[...].astype(F32)
        w = jnp.concatenate([w[i:i + 1] for i in range(w.shape[0])], axis=1)
        return _rb(jnp.sum(hn * w, axis=-1, keepdims=True))

    early = (n_seg - UNROLL - 1) * seg
    cp_early = pltpu.make_async_copy(out_v.at[pl.ds(0, early)], out_hbm.at[pl.ds(0, early)], sem_out[0])
    cp_late = pltpu.make_async_copy(out_v.at[pl.ds(early, S - early)],
                                    out_hbm.at[pl.ds(early, S - early)], sem_out[1])

    def finish_segment(sp, lane_id):
        rows = pl.ds(pl.multiple_of(sp * seg, seg), seg)
        h = _rb(x_v[sp].astype(F32) + _rb(acc_v[M:L, :]))
        hn = _layernorm(h)
        r = route(hn)
        h_v[rows, :] = h
        hn_v[rows, :] = hn
        out_v[rows, :] = (h + hn).astype(BF16)
        lane = lax.broadcasted_iota(jnp.int32, (seg, LANES), 1)
        r = jnp.where(lane == lane_id, r, scores())
        stage[r_at] = r.reshape(seg // HG, HG, LANES).astype(BF16)

    def step(s):
        lhs = jnp.concatenate([acc_v[0:M, :], xh_v[...]], axis=0).astype(BF16)
        norm_head(jnp.minimum(s + 1, n_seg - 1))
        qi = lax.broadcasted_iota(jnp.int32, (L, L), 0)
        ki = lax.broadcasted_iota(jnp.int32, (L, L), 1)
        visible = (qi < M) | (qi >= ki)

        def proj(m, h):
            j = m * H + h
            tail = stage[j // HG, (j % HG) * n_seg + s].astype(F32)
            return jnp.concatenate([_dot(lhs, w_tile(j)), tail], axis=0)

        val = {}
        acc = None
        for kind, h in _issue_order(H):
            if (kind, h) == ("q", 8):
                finish_segment(jnp.maximum(s - 1, 0), s - 1)
            if kind in "qkv":
                val[kind, h] = proj("qkv".index(kind), h)
            elif kind == "s":
                sc = _dot(val.pop(("q", h)), val.pop(("k", h)), NT) * (scale * LOG2E)
                sc = jnp.where(visible, sc, MASKED * LOG2E)
                ex = jnp.exp2(sc - jnp.max(sc, axis=-1, keepdims=True))
                val[kind, h] = ex, _recip(jnp.sum(ex, axis=-1, keepdims=True))
            elif kind == "p":
                ex, inv = val.pop(("s", h))
                val[kind, h] = _dot(ex, val.pop(("v", h))) * inv
            else:
                w = w_tile(3 * H + h)
                w = jnp.concatenate([w[t * Dh:(t + 1) * Dh] for t in range(n_col)], axis=1)
                y = _dot(val.pop(("p", h)), w)
                acc = y if acc is None else acc + y
        acc_v[...] = acc

    n_iter = n_seg // UNROLL

    def group(t, carry):
        pl.when(t == n_iter - 1)(cp_early.start)
        for u in range(UNROLL):
            step(t * UNROLL + u)
            for j in late[u::UNROLL - 1] if u < UNROLL - 1 else ():
                project_tail(j, jnp.minimum(t + 1, n_iter - 1))
        return carry

    lax.fori_loop(0, n_iter, group, 0)
    for cp in cp_ffn:
        cp.wait()
    finish_segment(n_seg - 1, n_seg - 1)
    cp_late.start()

    r = scores()
    pos = (lax.broadcasted_iota(jnp.int32, r.shape, 1) * seg
           + lax.broadcasted_iota(jnp.int32, r.shape, 0))
    last = seg * LANES - 1
    mag = (pltpu.bitcast(r, jnp.int32) >> 16) & 0x7FFF
    rank = jnp.where((r != r) | (pos >= S), 0, 0x8000 + jnp.where(r < 0, -mag, mag))
    key = pltpu.bitcast((1 << 30) + rank * (last + 1) + (last - pos), F32)
    key0 = jnp.max(key, keepdims=True)
    key1 = jnp.max(jnp.where(key == key0, 0.0, key), keepdims=True)
    i0, i1 = (jnp.clip(last - (lax.bitcast_convert_type(k, jnp.int32)[0, 0] & last), 0, S - 1)
              for k in (key0, key1))

    first = lax.broadcasted_iota(jnp.int32, (8, D), 0) == 0
    h_sel = jnp.where(first, h_v[pl.ds(i0, 1), :], h_v[pl.ds(i1, 1), :])
    hn_sel = jnp.where(first, hn_v[pl.ds(i0, 1), :], hn_v[pl.ds(i1, 1), :])
    r_sel = route(hn_sel)
    g = _rb(_dot(hn_sel, wg_v[...]))
    u = _rb(_dot(hn_sel, wu_v[...]))
    g = _rb(g * _rb(jax.nn.sigmoid(g)))
    y = _rb(_dot(_rb(g * u), wd_v[...]))
    y = _rb(y * _rb(jax.nn.sigmoid(r_sel)))
    new = h_sel + _rb(hn_sel + y)

    cp_early.wait()
    cp_late.wait()
    tile = 16
    fix = []
    for t, idx in enumerate((i0, i1)):
        start = pl.multiple_of((idx // tile) * tile, tile)
        rows = pl.ds(start, tile)
        hit = lax.broadcasted_iota(jnp.int32, (tile, D), 0) == idx - start
        out_v[rows, :] = jnp.where(hit, new[t:t + 1], out_v[rows, :].astype(F32)).astype(BF16)
        fix.append(pltpu.make_async_copy(out_v.at[rows], out_hbm.at[rows], sem_out[t]))
    two_tiles = i0 // tile != i1 // tile
    fix[0].start()
    pl.when(two_tiles)(fix[1].start)
    fix[0].wait()
    pl.when(two_tiles)(fix[1].wait)


@functools.partial(jax.jit, static_argnames=("A_seg_len",))
def pallas_sequential_preLN__memory_aug_recurrent_mem_tr__moe_arch_mod__prompt_kernel(
    A_x: jax.Array,
    A_mem0: jax.Array,
    A_Wq: jax.Array,
    A_Wk: jax.Array,
    A_Wv: jax.Array,
    A_Wo: jax.Array,
    A_seg_len: int,
    B_x: jax.Array,
    B_w_r: jax.Array,
    B_w_gate: jax.Array,
    B_w_up: jax.Array,
    B_w_down: jax.Array,
):
    del B_x
    B, S, D = A_x.shape
    M = A_mem0.shape[1]
    _, H, Dh = A_Wq.shape
    F = B_w_gate.shape[1]
    seg = int(A_seg_len)
    n_seg = S // seg
    assert (B, S, D, M, H, Dh, seg) == (1, 2048, 512, 8, 32, LANES, 32)

    hbm = pl.BlockSpec(memory_space=pl.ANY)
    n_chunk = 3 * (H // HG)
    out = pl.pallas_call(
        _kernel,
        out_shape=jax.ShapeDtypeStruct((S, D), BF16),
        in_specs=[hbm] * 10,
        out_specs=hbm,
        scratch_shapes=[
            pltpu.VMEM((n_seg, seg, D), BF16),
            pltpu.VMEM((M, D), BF16),
            pltpu.VMEM((D // LANES, LANES), BF16),
            pltpu.VMEM((D, F), BF16),
            pltpu.VMEM((D, F), BF16),
            pltpu.VMEM((F, D), BF16),
            pltpu.VMEM((n_seg, M, D), BF16),
            pltpu.VMEM((seg - M, D), F32),
            pltpu.VMEM((n_seg * M // 2, D), U32),
            pltpu.VMEM((n_chunk + 1, D, HG, Dh), BF16),
            pltpu.VMEM((2 * H // HG, HG, D // 2, Dh), U32),
            pltpu.VMEM((2 * H // HG, HG, D // 2, Dh), U32),
            pltpu.VMEM((H, Dh, D), BF16),
            pltpu.VMEM((M + seg, D), F32),
            pltpu.VMEM((S, D), F32),
            pltpu.VMEM((S, D), F32),
            pltpu.VMEM((S, D), BF16),
            pltpu.SemaphoreType.DMA((n_chunk + 2 * D // LANES,)),
            pltpu.SemaphoreType.DMA((9,)),
        ],
        compiler_params=pltpu.CompilerParams(vmem_limit_bytes=110 * 1024 * 1024),
        name="rmt_mod_block",
    )(
        A_x.reshape(n_seg, seg, D), A_mem0.reshape(M, D), A_Wq, A_Wk, A_Wv, A_Wo,
        B_w_r.reshape(D // LANES, LANES), B_w_gate, B_w_up, B_w_down,
    )
    return out.reshape(B, S, D)
```
